```python
import jax
import jax.numpy as jnp

def _softmax(x, axis=-1):
    return jax.nn.softmax(x, axis=axis)

def _gelu(x):
    return jax.nn.gelu(x, approximate=True)

def _silu(x):
    return jax.nn.silu(x)

def _sigmoid(x):
    return jax.nn.sigmoid(x)

def _layernorm(x, axis=-1, eps=1e-05):
    m = jnp.mean(x, axis=axis, keepdims=True)
    v = jnp.var(x, axis=axis, keepdims=True)
    return (x - m) / jnp.sqrt(v + eps)

def _scatter_add(tgt, idx, src, axis=0):
    return tgt.at[idx].add(src)

def _segment_sum(src, seg, n):
    return jax.ops.segment_sum(src, seg, n)

class _Rng:

    def __init__(self, key):
        self._k = key

    def _next(self):
        self._k, sub = jax.random.split(self._k)
        return sub

    def normal(self, shape):
        return jax.random.normal(self._next(), shape, dtype=jnp.bfloat16)

    def randint(self, lo, hi, shape):
        return jax.random.randint(self._next(), shape, lo, hi, dtype=jnp.int32)

    def uniform(self, shape, lo=0.0, hi=1.0):
        return jax.random.uniform(self._next(), shape, jnp.bfloat16, lo, hi)

    def permutation(self, n):
        return jax.random.permutation(self._next(), n)
kernel_name = 'adaLN_cond__sliding_block_cached__moe_arch_mod__decode'

def setup_inputs():
    _rng = _Rng(jax.random.key(int.from_bytes(__import__("os").urandom(4), "little")))
    _w = lambda a: (lambda t: t.astype(jnp.bfloat16) if jnp.issubdtype(t.dtype, jnp.floating) else t)(jnp.asarray(a))

    def _A_setup():
        B, Sq, D = (8, 1, 576)
        Hq, Hkv, Sk, Dh = (32, 16, 8192, 128)
        assert Hq % Hkv == 0, (Hq, Hkv)
        return {'x': _w((lambda *s: _rng.normal(s) * 0.05)(B, Sq, D)), 'k_cache': _w((lambda *s: _rng.normal(s) * 0.05)(B, Hkv, Sk, Dh)), 'v_cache': _w((lambda *s: _rng.normal(s) * 0.05)(B, Hkv, Sk, Dh)), 'wq': _w((lambda *s: _rng.normal(s) * 0.05)(D, Hq * Dh) * D ** (-0.5)), 'wo': _w((lambda *s: _rng.normal(s) * 0.05)(Hq * Dh, D) * (Hq * Dh) ** (-0.5))}
    _A_in = _A_setup()

    def _B_setup():
        B, S, D, F, C = (8, 1, 576, 4608, 1)
        return {'x': _w((lambda *s: _rng.normal(s) * 0.05)(B, S, D)), 'w_r': _w((lambda *s: _rng.normal(s) * 0.05)(D)), 'w_gate': _w((lambda *s: _rng.normal(s) * 0.05)(D, F)), 'w_up': _w((lambda *s: _rng.normal(s) * 0.05)(D, F)), 'w_down': _w((lambda *s: _rng.normal(s) * 0.05)(F, D))}
    _B_in = _B_setup()
    return {'A_x': _A_in['x'], 'A_k_cache': _A_in['k_cache'], 'A_v_cache': _A_in['v_cache'], 'A_wq': _A_in['wq'], 'A_wo': _A_in['wo'], 'B_x': _B_in['x'], 'B_w_r': _B_in['w_r'], 'B_w_gate': _B_in['w_gate'], 'B_w_up': _B_in['w_up'], 'B_w_down': _B_in['w_down'], 'c': _w((lambda *s: _rng.normal(s) * 0.05)(8, 576)), 'w_mod': _w((lambda *s: _rng.normal(s) * 0.05)(576, 6 * 576) * 576 ** (-0.5))}

def reference(A_x, A_k_cache, A_v_cache, A_wq, A_wo, B_x, B_w_r, B_w_gate, B_w_up, B_w_down, c, w_mod):

    def _A_ref(x, k_cache, v_cache, wq, wo):
        B, Sq, D = x.shape
        Hq, Dh = (32, 128)
        Hkv, Sk = (k_cache.shape[1], k_cache.shape[2])
        W = min(4096, max(256, Sk // 4))
        rep = Hq // Hkv
        q = (lambda x, *d: x.transpose(*d))((x @ wq).reshape(B, Sq, Hq, Dh), 0, 2, 1, 3)
        k = jnp.repeat(k_cache[:, :, Sk - W:, :], rep, axis=1)
        v = jnp.repeat(v_cache[:, :, Sk - W:, :], rep, axis=1)
        scores = jnp.einsum('bhqd,bhkd->bhqk', q, k) * Dh ** (-0.5)
        p = _softmax(scores, axis=-1)
        o = jnp.einsum('bhqk,bhkd->bhqd', p, v)
        return (lambda x, *d: x.transpose(*d))(o, 0, 2, 1, 3).reshape(B, Sq, Hq * Dh) @ wo

    def _B_ref(x, w_r, w_gate, w_up, w_down):
        B, S, D = x.shape
        C = 1
        r = x @ w_r
        idx = jnp.argsort(-r, axis=-1)[:, :C]
        idx_e = jnp.repeat(idx.reshape(B, C, 1), D, axis=2)
        x_sel = jnp.take_along_axis(x, idx_e, axis=1)
        g = _silu(x_sel @ w_gate)
        u = x_sel @ w_up
        y = g * u @ w_down
        r_sel = _sigmoid(jnp.take_along_axis(r, idx, axis=1))
        y = y * r_sel.reshape(B, C, 1)
        b_off = (jnp.arange(B) * S).reshape(B, 1)
        flat_idx = (idx + b_off).reshape(B * C)
        zero = (x * 0.0).reshape(B * S, D)
        upd = _scatter_add(zero, flat_idx, y.reshape(B * C, D), axis=0)
        return x + upd.reshape(B, S, D)
    x = A_x
    mod = (_silu(c) @ w_mod).reshape(c.shape[0], 6, 1, -1)
    sa, ca, ga, sb, cb, gb = (mod[:, 0].copy(), mod[:, 1].copy(), mod[:, 2].copy(), mod[:, 3].copy(), mod[:, 4].copy(), mod[:, 5].copy())
    h = _layernorm(x, axis=-1) * (1 + ca) + sa
    x = x + ga * _A_ref(h, A_k_cache, A_v_cache, A_wq, A_wo)
    h = _layernorm(x, axis=-1) * (1 + cb) + sb
    x = x + gb * _B_ref(h, B_w_r, B_w_gate, B_w_up, B_w_down)
    return x
```

```python
import functools

import jax
import jax.numpy as jnp
from jax import lax
import jax.experimental.pallas as pl
import jax.experimental.pallas.tpu as pltpu

F32 = jnp.float32
BF16 = jnp.bfloat16

HQ = 32
DH = 128
RING = 8
LAG_K = 6
V_OFF = 9
LAG_PV = 14
FG, BG = 0, 1


def _chunks(total, n):
    base = (total // n) // 16 * 16
    extra = (total - base * n) // 16
    sizes = [base + 16] * extra + [base] * (n - extra)
    offs = [sum(sizes[:i]) for i in range(n)]
    return list(zip(offs, sizes))


def _merge(a, b):
    out = []
    ia = ib = 0
    while ia < len(a) or ib < len(b):
        if ib >= len(b) or (ia < len(a) and ia * len(b) <= ib * len(a)):
            out.append(a[ia]); ia += 1
        else:
            out.append(b[ib]); ib += 1
    return out


def _layernorm(x, eps=1e-5):
    m = jnp.mean(x, axis=-1, keepdims=True)
    xc = x - m
    v = jnp.mean(xc * xc, axis=-1, keepdims=True)
    return xc * lax.rsqrt(v + eps)


def _dot(a, b):
    return jnp.dot(a, b, preferred_element_type=F32)


def _dot_nt(a, b):
    return lax.dot_general(a, b, (((1,), (1,)), ((), ())), preferred_element_type=F32)


def _kernel(x_hbm, k_hbm, v_hbm, wq_hbm, wo_hbm, wr_hbm, wg_hbm, wu_hbm, wd_hbm,
            c_hbm, wm_hbm, out_ref,
            x_v, c_v, wr_v, wm_v, wq_v, wo_v, wg_v, wu_v, wd_v, kbuf, vbuf,
            mod_s, h_s, q_s, s_s, p_s, l_s, o_s, acc_s, act_s,
            sem_small, sem_w, sem_k, sem_v, sem_d, *, W):
    B, HKV, SK, _ = k_hbm.shape
    D = x_v.shape[1]
    FF = wg_v.shape[1]
    NP = B * HKV
    NRB = D // 8
    kv_chunks = _chunks(W, 10)
    scale = DH ** -0.5
    S_MOD, S_Q, S_O, S_G, S_U = range(5)

    def kv_starts(hbm, buf, sem, p, prio):
        h = p // B
        b = p % B
        slot = p % RING

        def mk(off, n):
            def go():
                pltpu.make_async_copy(
                    hbm.at[b, h, pl.ds(SK - W + off, n), :],
                    buf.at[slot, pl.ds(off, n), :], sem.at[slot]).start(priority=prio)
            return go
        return [mk(off, n) for off, n in kv_chunks]

    def kv_wait(buf, sem, p):
        slot = p % RING
        pltpu.make_async_copy(buf.at[slot], buf.at[slot], sem.at[slot]).wait()

    def w_start(hbm, buf, sem, rb, part, nparts, prio):
        n = buf.shape[1] // nparts
        r = rb * 8
        if not isinstance(rb, int):
            r = pl.multiple_of(r, 8)

        def go():
            pltpu.make_async_copy(
                hbm.at[pl.ds(r, 8), pl.ds(part * n, n)],
                buf.at[pl.ds(r, 8), pl.ds(part * n, n)], sem).start(priority=prio)
        return go

    def w_group(hbm, buf, sem, g, prio):
        return [w_start(hbm, buf, sem, g * 8 + i, part, 2, prio)
                for i in range(8) for part in range(2)]

    def w_split(hbm, buf, sem, rb):
        return [w_start(hbm, buf, sem, rb, 0, 2, FG), w_start(hbm, buf, sem, rb, 1, 2, BG)]

    def w_wait(buf, sem):
        pltpu.make_async_copy(buf, buf, sem).wait()

    def run(thunks):
        for t in thunks:
            t()

    def slot_k_wo(t):
        return _merge(kv_starts(k_hbm, kbuf, sem_k, t, FG),
                      w_group(wo_hbm, wo_v, sem_w.at[S_O], t, BG))

    def slot_k_v(t):
        return _merge(kv_starts(k_hbm, kbuf, sem_k, t, FG),
                      kv_starts(v_hbm, vbuf, sem_v, t - V_OFF, BG))

    def slot_g_v(t):
        return _merge(w_group(wg_hbm, wg_v, sem_w.at[S_G], t - NP, FG),
                      kv_starts(v_hbm, vbuf, sem_v, t - V_OFF, BG))

    U_PER_SLOT = 12

    def slot_u(t):
        rb0 = (t - (NP + V_OFF)) * U_PER_SLOT
        return [th for i in range(U_PER_SLOT)
                for th in w_split(wu_hbm, wu_v, sem_w.at[S_U], rb0 + i)]

    small = [pltpu.make_async_copy(c_hbm, c_v, sem_small.at[0]),
             pltpu.make_async_copy(x_hbm, x_v, sem_small.at[1]),
             pltpu.make_async_copy(wr_hbm, wr_v, sem_small.at[2])]
    for cp in small:
        cp.start(priority=FG)

    def p0(i, carry):
        w_start(wm_hbm, wm_v, sem_w.at[S_MOD], i, 0, 1, FG)()
        w_start(wq_hbm, wq_v, sem_w.at[S_Q], i, 0, 2, BG)()
        w_start(wq_hbm, wq_v, sem_w.at[S_Q], i, 1, 2, BG)()
        return carry
    lax.fori_loop(0, NRB, p0, 0, unroll=4)

    run(slot_k_wo(0))
    for cp in small:
        cp.wait()
    w_wait(wm_v, sem_w.at[S_MOD])
    c = c_v[...].astype(F32)
    sc = (c * jax.nn.sigmoid(c)).astype(BF16)
    mod_a = _dot(sc, wm_v[:, 0:2 * D])
    x = x_v[...].astype(F32)
    h_s[...] = _layernorm(x) * (1.0 + mod_a[:, D:2 * D]) + mod_a[:, 0:D]

    run(slot_k_wo(1))
    w_wait(wq_v, sem_w.at[S_Q])
    hb = h_s[...].astype(BF16)
    NQ = 2
    for part in range(NQ):
        n = HQ * DH // NQ
        q = _dot(hb, wq_v[:, part * n:(part + 1) * n])
        for j in range(HQ // NQ):
            hq = part * (HQ // NQ) + j
            q_s[hq // 2, (hq % 2) * B:(hq % 2 + 1) * B, :] = q[:, j * DH:(j + 1) * DH]
        run(slot_k_wo(2 + part))
    mod_s[...] = _dot(sc, wm_v[:, 2 * D:6 * D])
    acc_s[...] = jnp.zeros_like(acc_s)
    for t in range(2 + NQ, LAG_K):
        run(slot_k_wo(t))

    row_s = lax.broadcasted_iota(jnp.int32, (2 * B, W), 0) % B
    row_o = lax.broadcasted_iota(jnp.int32, (2 * B, DH), 0) % B

    def issue(t, half):
        def sel(thunks):
            n = len(thunks) // 2
            return thunks[:n] if half == 0 else thunks[n:]

        @pl.when(t < V_OFF)
        def _():
            run(sel(slot_k_wo(t)))

        @pl.when(jnp.logical_and(t >= V_OFF, t < NP))
        def _():
            run(sel(slot_k_v(t)))

        @pl.when(jnp.logical_and(t >= NP, t < NP + V_OFF))
        def _():
            run(sel(slot_g_v(t)))

        @pl.when(t >= NP + V_OFF)
        def _():
            run(sel(slot_u(t)))

    def body(t, carry):
        @pl.when(t < NP + LAG_K)
        def _():
            p = t - LAG_K
            kv_wait(kbuf, sem_k, p)
            qh = q_s[p // B].astype(BF16)
            s = _dot_nt(qh, kbuf[p % RING])
            pltpu.store(s_s, s, mask=row_s == p % B)

        issue(t, 0)

        @pl.when(t >= LAG_PV)
        def _():
            p = t - LAG_PV
            kv_wait(vbuf, sem_v, p)
            o = _dot(p_s[...], vbuf[p % RING])
            pltpu.store(o_s, o, mask=row_o == p % B)

        issue(t, 1)

        @pl.when((t - LAG_K) % B == B - 1)
        def _():
            @pl.when(t >= LAG_PV)
            def _():
                h = (t - LAG_PV) // B

                @pl.when(h == 0)
                def _():
                    w_wait(wo_v, sem_w.at[S_O])
                o = (o_s[...] / l_s[...]).astype(BF16)
                o2 = jnp.concatenate([o[0:B], o[B:2 * B]], axis=1)
                col = pl.multiple_of(h * (2 * DH), 2 * DH)
                acc_s[...] += _dot_nt(o2, wo_v[:, pl.ds(col, 2 * DH)])

            @pl.when(t < NP + LAG_K)
            def _():
                s = s_s[...]
                m = jnp.max(s, axis=-1, keepdims=True)
                e = jnp.exp((s - m) * scale)
                l_s[...] = jnp.broadcast_to(jnp.sum(e, axis=-1, keepdims=True), l_s.shape)
                p_s[...] = e.astype(BF16)
        return carry

    T_END = NP + LAG_PV
    lax.fori_loop(LAG_K, T_END, body, 0)

    u_done = (T_END - NP - V_OFF) * U_PER_SLOT
    pending = [th for rb in range(u_done, NRB)
               for th in w_split(wu_hbm, wu_v, sem_w.at[S_U], rb)]
    d_groups = [(0, 128), (128, 128), (256, 128), (384, 128), (512, 64)]
    for gi, (r0, nr) in enumerate(d_groups):
        for rb in range(r0 // 8, (r0 + nr) // 8):
            pending += w_split(wd_hbm, wd_v, sem_d.at[gi], rb)
    pending = iter(pending)

    def issue_n(n):
        for _ in range(n):
            th = next(pending, None)
            if th is not None:
                th()

    mod = mod_s[...]
    ga, sb, cb, gb = (mod[:, i * D:(i + 1) * D] for i in range(4))
    x2 = x_v[...].astype(F32) + ga * acc_s[...]
    h2 = _layernorm(x2) * (1.0 + cb) + sb
    h2b = h2.astype(BF16)
    wr = wr_v[...].astype(F32).reshape(1, D)
    rsel = jax.nn.sigmoid(jnp.sum(h2 * wr, axis=-1, keepdims=True))
    issue_n(16)
    w_wait(wg_v, sem_w.at[S_G])
    NF = 3
    fn = FF // NF
    for j in range(NF):
        g = _dot(h2b, wg_v[:, j * fn:(j + 1) * fn])
        act_s[:, j * fn:(j + 1) * fn] = g * jax.nn.sigmoid(g)
        issue_n(16)
    w_wait(wu_v, sem_w.at[S_U])
    for j in range(NF):
        u = _dot(h2b, wu_v[:, j * fn:(j + 1) * fn])
        act_s[:, j * fn:(j + 1) * fn] = act_s[:, j * fn:(j + 1) * fn] * u
        issue_n(16)
    act = act_s[...].astype(BF16)
    ys = []
    for gi, (r0, nr) in enumerate(d_groups):
        issue_n(32)
        blk = wd_v.at[pl.ds(r0, nr), :]
        pltpu.make_async_copy(blk, blk, sem_d.at[gi]).wait()
        ys.append(_dot_nt(act, wd_v[r0:r0 + nr, :]))
    y = jnp.concatenate(ys, axis=1)
    out_ref[...] = (x2 + gb * (h2 + y * rsel)).astype(out_ref.dtype)


@jax.jit
def pallas_adaLN_cond__sliding_block_cached__moe_arch_mod__decode_kernel(
    A_x: jax.Array,
    A_k_cache: jax.Array,
    A_v_cache: jax.Array,
    A_wq: jax.Array,
    A_wo: jax.Array,
    B_x: jax.Array,
    B_w_r: jax.Array,
    B_w_gate: jax.Array,
    B_w_up: jax.Array,
    B_w_down: jax.Array,
    c: jax.Array,
    w_mod: jax.Array,
):
    B, SQ, D = A_x.shape
    _, HKV, SK, _ = A_k_cache.shape
    FF = B_w_gate.shape[1]
    W = min(4096, max(256, SK // 4))
    assert SQ == 1 and HQ == 2 * HKV and B == 8

    vm = pltpu.VMEM
    scratch = [
        vm((B, D), BF16), vm((B, D), BF16), vm((D,), BF16),
        vm((D, 6 * D), BF16), vm((D, HQ * DH), BF16), vm((D, HQ * DH), BF16),
        vm((D, FF), BF16), vm((D, FF), BF16), vm((D, FF), BF16),
        vm((RING, W, DH), BF16), vm((RING, W, DH), BF16),
        vm((B, 4 * D), F32),
        vm((B, D), F32),
        vm((HKV, 2 * B, DH), F32),
        vm((2 * B, W), F32),
        vm((2 * B, W), BF16),
        vm((2 * B, DH), F32),
        vm((2 * B, DH), F32),
        vm((B, D), F32),
        vm((B, FF), F32),
        pltpu.SemaphoreType.DMA((3,)),
        pltpu.SemaphoreType.DMA((5,)),
        pltpu.SemaphoreType.DMA((RING,)),
        pltpu.SemaphoreType.DMA((RING,)),
        pltpu.SemaphoreType.DMA((5,)),
    ]
    out = pl.pallas_call(
        functools.partial(_kernel, W=W),
        out_shape=jax.ShapeDtypeStruct((B, D), A_x.dtype),
        in_specs=[pl.BlockSpec(memory_space=pl.ANY)] * 11,
        out_specs=pl.BlockSpec(memory_space=pltpu.VMEM),
        scratch_shapes=scratch,
        compiler_params=pltpu.CompilerParams(
            vmem_limit_bytes=64 * 1024 * 1024,
            disable_bounds_checks=True,
            disable_semaphore_checks=True,
        ),
    )(A_x.reshape(B, D), A_k_cache, A_v_cache, A_wq, A_wo.T, B_w_r,
      B_w_gate, B_w_up, B_w_down.T, c, w_mod)
    return out.reshape(B, SQ, D)
```

```python
import functools

import jax
import jax.numpy as jnp
from jax import lax
import jax.experimental.pallas as pl
import jax.experimental.pallas.tpu as pltpu

F32 = jnp.float32
BF16 = jnp.bfloat16

HQ = 32
DH = 128
FG, BG = 0, 1
ST = 16

CFG = dict(scopes=False, ph_kv=16, ph_q=2, ph_f=8, ph_m=5, rot=2, bg_first=23, nsub0=4,
           gu0=16, gu_tail=2, ph_k=2, ph_v=4, ph_fin=5,
           tail_iss=(19, 19, 18, 22, 20, 6), post_iss=(8, 24, 24, 20, 100),
           d_fg=(0, 1), d_bg=(2, 3, 4), d_order=(0, 2, 1, 3, 4), it_m=2, it_q=4)

CFG.update({'tail_iss': (25, 25, 26, 32, 32, 6), 'post_iss': (10, 24, 24, 20, 100), 'gu_tail': 3, 'bg_first': 18})


class _NoScope:
    def __enter__(self): return self
    def __exit__(self, *a): return False


def scope(name):
    return jax.named_scope(name) if CFG['scopes'] else _NoScope()


def _merge(a, b):
    out = []
    ia = ib = 0
    while ia < len(a) or ib < len(b):
        if ib >= len(b) or (ia < len(a) and ia * len(b) <= ib * len(a)):
            out.append(a[ia]); ia += 1
        else:
            out.append(b[ib]); ib += 1
    return out


def _alternate(a, b):
    out = []
    for i in range(max(len(a), len(b))):
        if i < len(a): out.append(a[i])
        if i < len(b): out.append(b[i])
    return out


def _stripes(nrb, ntc, phase):
    nt = nrb * ntc
    out = []
    t = phase
    while t < nt + phase:
        t1 = min(t + ST, nt + phase)
        pcs = []
        while t < t1:
            rb, c = divmod(t, ntc)
            n = min(t1 - t, ntc - c)
            pcs.append((rb, c, n))
            t += n
        out.append(pcs)
    return out


def _substreams(lst, ns):
    per = -(-len(lst) // ns)
    return [lst[s * per + j] for j in range(per) for s in range(ns) if s * per + j < len(lst) and j < per]


def _layernorm(x, eps=1e-5):
    m = jnp.mean(x, axis=-1, keepdims=True)
    xc = x - m
    v = jnp.mean(xc * xc, axis=-1, keepdims=True)
    return xc * lax.rsqrt(v + eps)


def _dot(a, b):
    return jnp.dot(a, b, preferred_element_type=F32)


def _dot_nt(a, b):
    return lax.dot_general(a, b, (((1,), (1,)), ((), ())), preferred_element_type=F32)


def _kernel(x_hbm, k_hbm, v_hbm, wq_hbm, wo_hbm, wr_hbm, wg_hbm, wu_hbm, wd_hbm,
            c_hbm, wm_hbm, out_ref,
            x_v, c_v, wr_v, wm_v, wq_v, wo_v, wg_v, wu_v, wd_v, kbuf, vbuf,
            mod_s, h_s, q_s, s_s, p_s, l_s, o_s, acc_s, act_s, actb_s,
            sems, *, W):
    B, HKV, SK, _ = k_hbm.shape
    D = x_v.shape[1]
    FF = wg_v.shape[1]
    NRB = D // 8
    scale = DH ** -0.5
    S_C, S_X, S_R, S_MOD, S_Q, S_O, S_G, S_U, S_K, S_V, S_D = 0, 1, 2, 3, 4, 5, 6, 7, 8, 10, 12
    PH = CFG['ph_kv']
    NFULL = W // 128 - (1 if PH else 0)

    def w_stripe(hbm, buf, si, pcs, prio, rb0=0, nrb=NRB, base=0):
        sem = sems.at[si]

        def go():
            for rb, c, n in pcs:
                r = (base + (rb0 + rb) % nrb) * 8
                if not isinstance(r, int):
                    r = pl.multiple_of(r, 8)
                pltpu.make_async_copy(
                    hbm.at[pl.ds(r, 8), pl.ds(c * 128, n * 128)],
                    buf.at[pl.ds(r, 8), pl.ds(c * 128, n * 128)], sem).start(priority=prio)
        go.si = si
        return go

    def kv_round(g, r):
        slot = g % 2
        out = []
        for b in range(B):
            for hbm, buf, si, prio in ((k_hbm, kbuf, S_K, FG), (v_hbm, vbuf, S_V, BG)):
                if r is None:
                    pcs = [(0, PH), (W - 128 + PH, 128 - PH)]
                else:
                    pcs = [(pl.multiple_of(PH + ((r + CFG['rot'] * b) % NFULL) * 128, 8), 128)]

                def go(hbm=hbm, buf=buf, si=si, prio=prio, pcs=pcs, b=b):
                    for o, n in pcs:
                        pltpu.make_async_copy(
                            hbm.at[b, g, pl.ds(SK - W + o, n), :],
                            buf.at[slot, b, pl.ds(o, n), :], sems.at[si + slot]).start(priority=prio)
                out.append(go)
        return out

    def wait_all(ref, si):
        pltpu.make_async_copy(ref, ref, sems.at[si]).wait()

    def run(thunks):
        for t in thunks:
            t()

    def pairs(lst):
        return [lst[i:i + 2] for i in range(0, len(lst), 2)]

    def flat(ll):
        return [x for l in ll for x in l]

    st_m = [w_stripe(wm_hbm, wm_v, S_MOD, p, FG)
            for p in _substreams(_stripes(NRB, wm_v.shape[1] // 128, CFG['ph_m']), CFG['nsub0'])]
    st_q = [w_stripe(wq_hbm, wq_v, S_Q, p, BG)
            for p in _substreams(_stripes(NRB, wq_v.shape[1] // 128, CFG['ph_q']), CFG['nsub0'])]
    small = [pltpu.make_async_copy(c_hbm, c_v, sems.at[S_C]),
             pltpu.make_async_copy(x_hbm, x_v, sems.at[S_X]),
             pltpu.make_async_copy(wr_hbm, wr_v, sems.at[S_R])]
    with scope('p0'):
        run(st_q[:CFG['bg_first']])
        for cp in small:
            cp.start(priority=FG)
        run(_alternate(st_m, st_q[CFG['bg_first']:]))

    NTF = FF // 128
    per_f = _stripes(4, NTF, CFG['ph_f'])
    NPER = NRB // 4

    def gu_period(p):
        return _alternate(
            [w_stripe(wg_hbm, wg_v, S_G, pc, FG, rb0=p * 4) for pc in per_f],
            [w_stripe(wu_hbm, wu_v, S_U, pc, BG, rb0=p * 4) for pc in per_f])

    d_groups = [(0, 128), (128, 128), (256, 128), (384, 128), (512, 64)]

    def d_list(gs, prio):
        return [w_stripe(wd_hbm, wd_v, S_D + gi, pc, prio, nrb=d_groups[gi][1] // 8, base=d_groups[gi][0] // 8)
                for gi in gs for pc in _stripes(d_groups[gi][1] // 8, NTF, CFG['ph_f'])]

    tail = flat([gu_period(p) for p in range(NPER - CFG['gu_tail'], NPER)])
    tail += _alternate(d_list(CFG['d_fg'], FG), d_list(CFG['d_bg'], BG))

    def take(n):
        out = tail[:n]
        del tail[:n]
        return out

    def flush(si):
        idx = [i for i, t in enumerate(tail) if t.si == si]
        if idx:
            run(take(idx[-1] + 1))

    row_s = lax.broadcasted_iota(jnp.int32, (2 * B, W), 0) % B
    row_o = lax.broadcasted_iota(jnp.int32, (2 * B, DH), 0) % B
    NIT = HKV * 8
    per_o = _stripes(4, wo_v.shape[1] // 128, CFG['ph_q'])
    N_WO = NRB // 8
    GU0 = CFG['gu0']
    GU1 = GU0 + NPER - CFG['gu_tail']
    tail_lists = [take(n) for n in CFG['tail_iss']]
    T_END = NIT + len(tail_lists)
    assert len(tail_lists) == CFG['ph_fin'] + 1

    def issue(it):
        g = it // 8
        r0 = (it % 8) * 2

        def kv(extra):
            ex = pairs(extra)
            ex0, ex1 = ex[:len(ex) // 2], ex[len(ex) // 2:]
            run(flat(_merge(pairs(kv_round(g, r0)), ex0)))
            if PH:
                @pl.when(r0 + 1 < NFULL)
                def _():
                    run(flat(_merge(pairs(kv_round(g, r0 + 1)), ex1)))

                @pl.when(r0 + 1 == NFULL)
                def _():
                    run(flat(_merge(pairs(kv_round(g, None)), ex1)))
            else:
                run(flat(_merge(pairs(kv_round(g, r0 + 1)), ex1)))

        is_wo = it < N_WO
        is_gu = jnp.logical_and(it >= GU0, it < GU1)

        @pl.when(is_wo)
        def _():
            kv(_alternate(
                [w_stripe(wo_hbm, wo_v, S_O, pc, FG, rb0=it * 4) for pc in per_o],
                [w_stripe(wo_hbm, wo_v, S_O, pc, BG, rb0=(it + N_WO) * 4) for pc in per_o]))

        @pl.when(is_gu)
        def _():
            kv(gu_period(it - GU0))

        @pl.when(jnp.logical_and(it < NIT, jnp.logical_not(jnp.logical_or(is_wo, is_gu))))
        def _():
            kv([])

        for k, lst in enumerate(tail_lists):
            @pl.when(it == NIT + k)
            def _(lst=lst):
                run(lst)

    def body(it, carry):
        ph = it % 8
        g = it // 8 - 1
        slot = (g + 2) % 2

        @pl.when(it == CFG['it_m'])
        def _():
            for cp in small:
                cp.wait()
            wait_all(wm_v, S_MOD)
            c = c_v[...].astype(F32)
            sc = (c * jax.nn.sigmoid(c)).astype(BF16)
            mod = _dot(sc, wm_v[...])
            x = x_v[...].astype(F32)
            h_s[...] = _layernorm(x) * (1.0 + mod[:, D:2 * D]) + mod[:, 0:D]
            mod_s[...] = mod[:, 2 * D:6 * D]
            acc_s[...] = jnp.zeros_like(acc_s)

        @pl.when(it == CFG['it_q'])
        def _():
            wait_all(wq_v, S_Q)
            q = _dot(h_s[...].astype(BF16), wq_v[...])
            for hq in range(HQ):
                q_s[hq // 2, (hq % 2) * B:(hq % 2 + 1) * B, :] = q[:, hq * DH:(hq + 1) * DH]

        @pl.when(g >= 0)
        def _():
            @pl.when(ph == CFG['ph_k'])
            def _():
                wait_all(kbuf.at[slot], S_K + slot)

            @pl.when(jnp.logical_or(ph == CFG['ph_k'], ph == CFG['ph_k'] + 1))
            def _():
                qh = q_s[g].astype(BF16)

                def qk(j, c):
                    b = (ph - CFG['ph_k']) * (B // 2) + j
                    pltpu.store(s_s, _dot_nt(qh, kbuf[slot, b]), mask=row_s == b)
                    return c
                lax.fori_loop(0, B // 2, qk, 0)

            @pl.when(ph == CFG['ph_k'] + 1)
            def _():
                s = s_s[...]
                m = jnp.max(s, axis=-1, keepdims=True)
                e = jnp.exp((s - m) * scale)
                l_s[...] = jnp.broadcast_to(jnp.sum(e, axis=-1, keepdims=True), l_s.shape)
                p_s[...] = e.astype(BF16)

            @pl.when(ph == CFG['ph_v'])
            def _():
                wait_all(vbuf.at[slot], S_V + slot)
                pb = p_s[...]

                def pv(j, o):
                    for jj in range(2):
                        b = 2 * j + jj
                        o = jnp.where(row_o == b, _dot(pb, vbuf[slot, b]), o)
                    return o
                o_s[...] = lax.fori_loop(0, B // 2, pv, jnp.zeros((2 * B, DH), F32))

            @pl.when(ph == CFG['ph_fin'])
            def _():
                @pl.when(g == 0)
                def _():
                    wait_all(wo_v, S_O)
                o = (o_s[...] / l_s[...]).astype(BF16)
                o2 = jnp.concatenate([o[0:B], o[B:2 * B]], axis=1)
                col = pl.multiple_of(g * (2 * DH), 2 * DH)
                acc_s[...] += _dot_nt(o2, wo_v[:, pl.ds(col, 2 * DH)])

        issue(it)
        return carry

    if CFG['scopes']:
        for nm, a, b in [('loopA', 0, 16), ('loopB', 16, 40), ('loopC', 40, NIT)] + [('t%d' % k, NIT + k, NIT + k + 1) for k in range(len(tail_lists))]:
            with scope(nm):
                lax.fori_loop(a, b, body, 0)
    else:
        lax.fori_loop(0, T_END, body, 0)

    post = list(CFG['post_iss'])

    def issue_post():
        run(take(post.pop(0) if post else 1000))

    mod = mod_s[...]
    ga, sb, cb, gb = (mod[:, i * D:(i + 1) * D] for i in range(4))
    x2 = x_v[...].astype(F32) + ga * acc_s[...]
    h2 = _layernorm(x2) * (1.0 + cb) + sb
    h2b = h2.astype(BF16)
    wr = wr_v[...].astype(F32).reshape(1, D)
    rsel = jax.nn.sigmoid(jnp.sum(h2 * wr, axis=-1, keepdims=True))
    acc_s[...] = x2 + gb * h2
    h_s[...] = gb * rsel
    flush(S_G)
    with scope('waitg'):
        wait_all(wg_v, S_G)
    issue_post()
    g = _dot(h2b, wg_v[...])
    act_s[...] = g * jax.nn.sigmoid(g)
    flush(S_U)
    with scope('waitu'):
        wait_all(wu_v, S_U)
    issue_post()
    u = _dot(h2b, wu_v[...])
    actb_s[...] = (act_s[...] * u).astype(BF16)
    for gi in CFG['d_order']:
        r0, nr = d_groups[gi]
        flush(S_D + gi)
        with scope('waitd%d' % gi):
            wait_all(wd_v.at[pl.ds(r0, nr), :], S_D + gi)
        issue_post()
        y = _dot_nt(actb_s[...], wd_v[r0:r0 + nr, :])
        out_ref[:, r0:r0 + nr] = (acc_s[:, r0:r0 + nr] + h_s[:, r0:r0 + nr] * y).astype(out_ref.dtype)


@jax.jit
def pallas_adaLN_cond__sliding_block_cached__moe_arch_mod__decode_kernel(
    A_x, A_k_cache, A_v_cache, A_wq, A_wo, B_x, B_w_r, B_w_gate, B_w_up, B_w_down, c, w_mod):
    B, SQ, D = A_x.shape
    _, HKV, SK, _ = A_k_cache.shape
    FF = B_w_gate.shape[1]
    W = min(4096, max(256, SK // 4))
    assert SQ == 1 and HQ == 2 * HKV and B == 8

    vm = pltpu.VMEM
    scratch = [
        vm((B, D), BF16), vm((B, D), BF16), vm((D,), BF16),
        vm((D, 6 * D), BF16), vm((D, HQ * DH), BF16), vm((D, HQ * DH), BF16),
        vm((D, FF), BF16), vm((D, FF), BF16), vm((D, FF), BF16),
        vm((2, B, W, DH), BF16), vm((2, B, W, DH), BF16),
        vm((B, 4 * D), F32),
        vm((B, D), F32),
        vm((HKV, 2 * B, DH), F32),
        vm((2 * B, W), F32),
        vm((2 * B, W), BF16),
        vm((2 * B, DH), F32),
        vm((2 * B, DH), F32),
        vm((B, D), F32),
        vm((B, FF), F32),
        vm((B, FF), BF16),
        pltpu.SemaphoreType.DMA((12 + 5,)),
    ]
    out = pl.pallas_call(
        functools.partial(_kernel, W=W),
        out_shape=jax.ShapeDtypeStruct((B, D), A_x.dtype),
        in_specs=[pl.BlockSpec(memory_space=pl.ANY)] * 11,
        out_specs=pl.BlockSpec(memory_space=pltpu.VMEM),
        scratch_shapes=scratch,
        compiler_params=pltpu.CompilerParams(
            vmem_limit_bytes=64 * 1024 * 1024,
            disable_bounds_checks=True,
            disable_semaphore_checks=True,
        ),
    )(A_x.reshape(B, D), A_k_cache, A_v_cache, A_wq, A_wo.T, B_w_r,
      B_w_gate, B_w_up, B_w_down.T, c, w_mod)
    return out.reshape(B, SQ, D)
```

```python
import functools

import jax
import jax.numpy as jnp
from jax import lax
import jax.experimental.pallas as pl
import jax.experimental.pallas.tpu as pltpu

F32 = jnp.float32
BF16 = jnp.bfloat16

HQ = 32
DH = 128
FG, BG = 0, 1
ST = 16

CFG = dict(scopes=False, ph_kv=144, ph_q=18, ph_f=24, ph_m=21, lag=25, lag_w=25,
           gu_tail=16, nsub=dict(M=2, Q=2, O=2, G=2, U=2), vb=4,
           fin=dict(G=64, U=52, B0=27, B1=18, B2=9, B3=0), tsub=2,
           c_split=(24, 12), c_w=256,
           tail_iss=(30, 30, 34, 40, 40, 8), post_iss=(14, 40, 100),
           ph_k=2, ph_v=4, ph_fin=5, it_m=2, it_q=4, qk_unroll=1, pv_unroll=2)


class _NoScope:
    def __enter__(self): return self
    def __exit__(self, *a): return False


def scope(name):
    return jax.named_scope(name) if CFG['scopes'] else _NoScope()


def _pieces(t, t1, ntc):
    pcs = []
    while t < t1:
        rb, c = divmod(t, ntc)
        n = min(t1 - t, ntc - c)
        pcs.append((rb, c, n))
        t += n
    return pcs


def _blocks(rb0, rb1, ntc, phase):
    lo, hi = rb0 * ntc, rb1 * ntc
    t = lo - ((lo - phase) % (2 * ST))
    out = []
    while t < hi:
        out.append([_pieces(max(t, lo), min(t + ST, hi), ntc),
                    _pieces(max(t + ST, lo), min(t + 2 * ST, hi), ntc)])
        t += 2 * ST
    sz = lambda b: sum(n for h in b for _, _, n in h)
    if len(out) > 2 and sz(out[0]) + sz(out[-1]) <= 2 * ST + 4:
        first, last = out.pop(0), out.pop()
        a, b = first[0] + first[1], last[0] + last[1]
        def join(p):
            q = []
            for x in p:
                if q and q[-1][0] == x[0] and q[-1][1] + q[-1][2] == x[1]:
                    q[-1] = (x[0], q[-1][1], q[-1][2] + x[2])
                else:
                    q.append(x)
            return q
        out.insert(0, [join(a), join(b)])
    return out


def _spread(streams):
    keyed = []
    for si, (items, fin) in enumerate(streams):
        for i, x in enumerate(items):
            keyed.append(((i + (si + 1.0) / (len(streams) + 1)) / len(items) * fin, si, i, x))
    keyed.sort(key=lambda z: z[:3])
    return [z[3] for z in keyed]


def _deadline(streams):
    rem = [list(it) for it, _ in streams]
    total = sum(len(r) for r in rem)
    last_used = [-1] * len(streams)
    out = []
    for k in range(total):
        el = [s for s in range(len(streams)) if rem[s] and streams[s][1] <= k]
        if not el:
            el = [min((s for s in range(len(streams)) if rem[s]), key=lambda s: streams[s][1])]
        s = min(el, key=lambda s: (last_used[s], -len(rem[s])))
        last_used[s] = k
        out.append(rem[s].pop())
    return out[::-1]


def _layernorm(x, eps=1e-5):
    m = jnp.mean(x, axis=-1, keepdims=True)
    xc = x - m
    v = jnp.mean(xc * xc, axis=-1, keepdims=True)
    return xc * lax.rsqrt(v + eps)


def _dot(a, b):
    return jnp.dot(a, b, preferred_element_type=F32)


def _dot_nt(a, b):
    return lax.dot_general(a, b, (((1,), (1,)), ((), ())), preferred_element_type=F32)


def _kernel(x_hbm, k_hbm, v_hbm, wq_hbm, wo_hbm, wr_hbm, wg_hbm, wu_hbm, wd_hbm,
            c_hbm, wm_hbm, out_ref,
            x_v, c_v, wr_v, wm_v, wq_v, wo_v, wg_v, wu_v, wd_v, kbuf, vbuf,
            mod_s, h_s, q_s, s_s, p_s, l_s, o_s, acc_s, act_s, actb_s,
            sems, *, W):
    B, HKV, SK, _ = k_hbm.shape
    D = x_v.shape[1]
    FF = wg_v.shape[1]
    NRB = D // 8
    NTF = FF // 128
    scale = DH ** -0.5
    S_C, S_X, S_R, S_MOD, S_Q, S_O, S_G, S_U, S_K, S_V, S_D = 0, 1, 2, 3, 4, 5, 6, 7, 8, 10, 12
    LAG = CFG['lag']
    NIT = HKV * 8

    def dma(src, dst, si, prio):
        def go():
            pltpu.make_async_copy(src(), dst(), sems.at[si]).start(priority=prio)
        go.si = si
        return go

    def w_pairs(hbm, buf, si, rb0, rb1, phase):
        def mk(pc, prio):
            rb, c, n = pc
            idx = (pl.ds(rb * 8, 8), pl.ds(c * 128, n * 128))
            return dma(lambda: hbm.at[idx], lambda: buf.at[idx], si, prio)
        return [([mk(p, FG) for p in f], [mk(p, BG) for p in b])
                for f, b in _blocks(rb0, rb1, buf.shape[1] // 128, phase)]

    PH = CFG['ph_kv']
    NJ = W // 256
    if PH % 256:
        kv_geo = [((0, PH), (PH + 256 * (NJ - 1), 256 - PH))]
        kv_geo += [((PH + 256 * j, 128), (PH + 256 * j + 128, 128)) for j in range(NJ - 1)]
    else:
        kv_geo = [((256 * j, 128), (256 * j + 128, 128)) for j in range(NJ)]

    def kv_half(rnd, p, half):
        j, isv = p // 2, p % 2
        hbm, buf, si = ((k_hbm, kbuf, S_K), (v_hbm, vbuf, S_V))[isv]
        o, n = kv_geo[j][half]
        g = rnd // 8
        b = (j + isv * CFG['vb'] + 8 - rnd % 8) % 8
        slot = g % 2
        return dma(lambda: hbm.at[b, g, pl.ds(SK - W + o, n), :],
                   lambda: buf.at[slot, b, pl.ds(o, n), :], si + slot, (FG, BG)[half])

    def lagged(pairs, pre_fg, post_bg, lag):
        bgs, at = [], {}
        for i, f in enumerate(pre_fg):
            at.setdefault(lag - len(pre_fg) + i if False else i, []).append(f)
        for f, b in pairs:
            at.setdefault(len(bgs) + lag, []).extend(f)
            bgs.extend(b)
        bgs.extend(post_bg)
        out = []
        for i in range(max(len(bgs), max(at) + 1)):
            out.extend(at.get(i, []))
            if i < len(bgs):
                out.append(bgs[i])
        return out

    def wait_all(ref, si):
        pltpu.make_async_copy(ref, ref, sems.at[si]).wait()

    def run(thunks):
        for t in thunks:
            t()

    RT = NRB - CFG['gu_tail']

    def subs(pairs_fn, rb1, ns):
        cuts = [rb1 * i // ns for i in range(ns + 1)]
        return [(pairs_fn(cuts[i], cuts[i + 1]), 1.0) for i in range(ns)]

    ns = CFG['nsub']
    streams = (subs(lambda a, b: w_pairs(wm_hbm, wm_v, S_MOD, a, b, CFG['ph_m']), NRB, ns['M'])
               + subs(lambda a, b: w_pairs(wq_hbm, wq_v, S_Q, a, b, CFG['ph_q']), NRB, ns['Q'])
               + subs(lambda a, b: w_pairs(wo_hbm, wo_v, S_O, a, b, CFG['ph_q']), NRB, ns['O'])
               + subs(lambda a, b: w_pairs(wg_hbm, wg_v, S_G, a, b, CFG['ph_f']), RT, ns['G'])
               + subs(lambda a, b: w_pairs(wu_hbm, wu_v, S_U, a, b, CFG['ph_f']), RT, ns['U']))
    streams = streams[0::2] + streams[1::2]
    small = [pltpu.make_async_copy(c_hbm, c_v, sems.at[S_C]),
             pltpu.make_async_copy(x_hbm, x_v, sems.at[S_X]),
             pltpu.make_async_copy(wr_hbm, wr_v, sems.at[S_R])]
    head = lagged(_spread(streams), [], [kv_half(n // 16, n % 16, 1) for n in range(LAG)], CFG['lag_w'])
    with scope('p0'):
        run(head[:40])
        for cp in small:
            cp.start(priority=FG)
        run(head[40:])

    fin = CFG['fin']
    d_rows = {'B%d' % k: (128 * k, 128 * (k + 1)) for k in range(4)}
    regions = sorted(d_rows, key=lambda nm: -fin[nm])
    def halves(pairs, key):
        n = CFG['tsub']
        return [(pairs[len(pairs) * i // n:len(pairs) * (i + 1) // n], fin[key]) for i in range(n)]
    streams = (halves(w_pairs(wg_hbm, wg_v, S_G, RT, NRB, CFG['ph_f']), 'G')
               + halves(w_pairs(wu_hbm, wu_v, S_U, RT, NRB, CFG['ph_f']), 'U'))
    for i, nm in enumerate(regions):
        streams += halves(w_pairs(wd_hbm, wd_v, S_D + i, d_rows[nm][0] // 8, d_rows[nm][1] // 8, CFG['ph_f']), nm)
    d_cols = {}
    last = []
    c0 = 0
    for i, n in enumerate(CFG['c_split']):
        nm = 'C%d' % i
        d_rows[nm] = (512, D)
        d_cols[nm] = (c0, c0 + n * 128)
        for c in range(c0, c0 + n * 128, CFG['c_w']):
            idx = (pl.ds(512, D - 512), pl.ds(c, min(CFG['c_w'], c0 + n * 128 - c)))
            last.append(dma(lambda idx=idx: wd_hbm.at[idx], lambda idx=idx: wd_v.at[idx], S_D + len(regions), BG))
        regions.append(nm)
        c0 += n * 128
    assert c0 == FF
    NPEEL = 2
    n0 = (NIT - NPEEL) * 16
    peel = []
    for n in range(n0, NIT * 16 - LAG):
        peel += [kv_half(n // 16, n % 16, 0), kv_half((n + LAG) // 16, (n + LAG) % 16, 1)]
    tail = peel + lagged(_deadline(streams), [kv_half(n // 16, n % 16, 0) for n in range(NIT * 16 - LAG, NIT * 16)], last, CFG['lag_w'])

    def take(n):
        out = tail[:n]
        del tail[:n]
        return out

    def flush(si):
        idx = [i for i, t in enumerate(tail) if t.si == si]
        if idx:
            run(take(idx[-1] + 1))

    row_s = lax.broadcasted_iota(jnp.int32, (2 * B, W), 0) % B
    row_o = lax.broadcasted_iota(jnp.int32, (2 * B, DH), 0) % B
    nkv = max(i for i, t in enumerate(tail) if S_K <= t.si < S_D) + 1
    tail_lists = [take(32), take(nkv - 32)]
    tail_lists += [take(n) for n in CFG['tail_iss']]
    T_END = NIT - NPEEL + len(tail_lists)
    assert len(CFG['tail_iss']) == CFG['ph_fin'] + 1

    def issue(it):
        @pl.when(it < NIT - NPEEL)
        def _():
            for p in range(16):
                kv_half(it, p, 0)()
                kv_half(it + (p + LAG) // 16, (p + LAG) % 16, 1)()

        @pl.when(it >= NIT - NPEEL)
        def _():
            for k, lst in enumerate(tail_lists):
                @pl.when(it == NIT - NPEEL + k)
                def _(lst=lst):
                    run(lst)

    def body(it, carry):
        ph = it % 8
        g = it // 8 - 1
        slot = (g + 2) % 2

        @pl.when(it == CFG['it_m'])
        def _():
            for cp in small:
                cp.wait()
            wait_all(wm_v, S_MOD)
            c = c_v[...].astype(F32)
            sc = (c * jax.nn.sigmoid(c)).astype(BF16)
            mod = _dot(sc, wm_v[...])
            x = x_v[...].astype(F32)
            h_s[...] = _layernorm(x) * (1.0 + mod[:, D:2 * D]) + mod[:, 0:D]
            mod_s[...] = mod[:, 2 * D:6 * D]
            acc_s[...] = jnp.zeros_like(acc_s)

        @pl.when(it == CFG['it_q'])
        def _():
            wait_all(wq_v, S_Q)
            wait_all(wo_v, S_O)
            q = _dot(h_s[...].astype(BF16), wq_v[...])
            for hq in range(HQ):
                q_s[hq // 2, (hq % 2) * B:(hq % 2 + 1) * B, :] = q[:, hq * DH:(hq + 1) * DH]

        @pl.when(g >= 0)
        def _():
            @pl.when(ph == CFG['ph_k'])
            def _():
                wait_all(kbuf.at[slot], S_K + slot)

            @pl.when(jnp.logical_or(ph == CFG['ph_k'], ph == CFG['ph_k'] + 1))
            def _():
                qh = q_s[g].astype(BF16)
                U = CFG['qk_unroll']

                def qk(j, c):
                    for jj in range(U):
                        b = (ph - CFG['ph_k']) * (B // 2) + j * U + jj
                        pltpu.store(s_s, _dot_nt(qh, kbuf[slot, b]), mask=row_s == b)
                    return c
                lax.fori_loop(0, B // 2 // U, qk, 0)

            @pl.when(ph == CFG['ph_k'] + 1)
            def _():
                s = s_s[...]
                m = jnp.max(s, axis=-1, keepdims=True)
                e = jnp.exp((s - m) * scale)
                l_s[...] = jnp.broadcast_to(jnp.sum(e, axis=-1, keepdims=True), l_s.shape)
                p_s[...] = e.astype(BF16)

            @pl.when(ph == CFG['ph_v'])
            def _():
                wait_all(vbuf.at[slot], S_V + slot)
                pb = p_s[...]
                U = CFG['pv_unroll']

                def pv(j, o):
                    for jj in range(U):
                        b = U * j + jj
                        o = jnp.where(row_o == b, _dot(pb, vbuf[slot, b]), o)
                    return o
                o_s[...] = lax.fori_loop(0, B // U, pv, jnp.zeros((2 * B, DH), F32))

            @pl.when(ph == CFG['ph_fin'])
            def _():
                o = (o_s[...] / l_s[...]).astype(BF16)
                o2 = jnp.concatenate([o[0:B], o[B:2 * B]], axis=1)
                col = pl.multiple_of(g * (2 * DH), 2 * DH)
                acc_s[...] += _dot_nt(o2, wo_v[:, pl.ds(col, 2 * DH)])

        issue(it)
        return carry

    if CFG['scopes']:
        for nm, a, b in [('loopA', 0, 16), ('loopB', 16, NIT - NPEEL)] + [('t%d' % k, NIT - NPEEL + k, NIT - NPEEL + k + 1) for k in range(len(tail_lists))]:
            with scope(nm):
                lax.fori_loop(a, b, body, 0)
    else:
        lax.fori_loop(0, T_END, body, 0)

    post = list(CFG['post_iss'])

    def issue_post():
        run(take(post.pop(0) if post else 1000))

    mod = mod_s[...]
    ga, sb, cb, gb = (mod[:, i * D:(i + 1) * D] for i in range(4))
    x2 = x_v[...].astype(F32) + ga * acc_s[...]
    h2 = _layernorm(x2) * (1.0 + cb) + sb
    h2b = h2.astype(BF16)
    wr = wr_v[...].astype(F32).reshape(1, D)
    rsel = jax.nn.sigmoid(jnp.sum(h2 * wr, axis=-1, keepdims=True))
    acc_s[...] = x2 + gb * h2
    h_s[...] = gb * rsel
    flush(S_G)
    with scope('waitg'):
        wait_all(wg_v, S_G)
    issue_post()
    g = _dot(h2b, wg_v[...])
    act_s[...] = g * jax.nn.sigmoid(g)
    flush(S_U)
    with scope('waitu'):
        wait_all(wu_v, S_U)
    issue_post()
    u = _dot(h2b, wu_v[...])
    actb_s[...] = (act_s[...] * u).astype(BF16)
    for ri, nm in enumerate(regions):
        r0, r1 = d_rows[nm]
        f0, f1 = d_cols.get(nm, (0, FF))
        flush(S_D + ri)
        with scope('wait' + nm):
            wait_all(wd_v.at[pl.ds(r0, r1 - r0), pl.ds(f0, f1 - f0)], S_D + ri)
        issue_post()
        y = _dot_nt(actb_s[:, f0:f1], wd_v[r0:r1, f0:f1])
        val = acc_s[:, r0:r1] + h_s[:, r0:r1] * y
        if f1 < FF:
            acc_s[:, r0:r1] = val
        else:
            out_ref[:, r0:r1] = val.astype(out_ref.dtype)
    assert not tail


@jax.jit
def pallas_adaLN_cond__sliding_block_cached__moe_arch_mod__decode_kernel(
    A_x, A_k_cache, A_v_cache, A_wq, A_wo, B_x, B_w_r, B_w_gate, B_w_up, B_w_down, c, w_mod):
    B, SQ, D = A_x.shape
    _, HKV, SK, _ = A_k_cache.shape
    FF = B_w_gate.shape[1]
    W = min(4096, max(256, SK // 4))
    assert SQ == 1 and HQ == 2 * HKV and B == 8

    vm = pltpu.VMEM
    scratch = [
        vm((B, D), BF16), vm((B, D), BF16), vm((D,), BF16),
        vm((D, 6 * D), BF16), vm((D, HQ * DH), BF16), vm((D, HQ * DH), BF16),
        vm((D, FF), BF16), vm((D, FF), BF16), vm((D, FF), BF16),
        vm((2, B, W, DH), BF16), vm((2, B, W, DH), BF16),
        vm((B, 4 * D), F32),
        vm((B, D), F32),
        vm((HKV, 2 * B, DH), F32),
        vm((2 * B, W), F32),
        vm((2 * B, W), BF16),
        vm((2 * B, DH), F32),
        vm((2 * B, DH), F32),
        vm((B, D), F32),
        vm((B, FF), F32),
        vm((B, FF), BF16),
        pltpu.SemaphoreType.DMA((12 + 8,)),
    ]
    out = pl.pallas_call(
        functools.partial(_kernel, W=W),
        out_shape=jax.ShapeDtypeStruct((B, D), A_x.dtype),
        in_specs=[pl.BlockSpec(memory_space=pl.ANY)] * 11,
        out_specs=pl.BlockSpec(memory_space=pltpu.VMEM),
        scratch_shapes=scratch,
        compiler_params=pltpu.CompilerParams(
            vmem_limit_bytes=64 * 1024 * 1024,
            disable_bounds_checks=True,
            disable_semaphore_checks=True,
        ),
    )(A_x.reshape(B, D), A_k_cache, A_v_cache, A_wq, A_wo.T, B_w_r,
      B_w_gate, B_w_up, B_w_down.T, c, w_mod)
    return out.reshape(B, SQ, D)
```

```python
import functools

import jax
import jax.numpy as jnp
from jax import lax
import jax.experimental.pallas as pl
import jax.experimental.pallas.tpu as pltpu

F32 = jnp.float32
BF16 = jnp.bfloat16

HQ = 32
DH = 128
FG, BG = 0, 1
ST = 16
GP = 8
RS = 16

CFG = dict(scopes=False, ph_kv=144, ph_q=18, ph_f=24, ph_m=21, lag=26, wlag=4,
           gu_tail=16, nsub=dict(M=2, Q=2, O=2, G=2, U=2), vb=4, tb=4,
           fin=dict(G=64, U=52, B0=27, B1=18, B2=9, B3=0), tsub=2,
           c_split=(24, 12), c_w=256, pad=0,
           qk_unroll=2, pv_unroll=4, sm_at=1, pv_at=2, tail_qk=((0, 1, 2, 3), (4, 5, 6, 7)), tail_pv=((0, 1, 2, 3, 4, 5, 6, 7),), tail_adv=(1, 0, 2, 1),
           post=(1, 2, 2, 1, 1, 1, 1, 1))


class _NoScope:
    def __enter__(self): return self
    def __exit__(self, *a): return False


def scope(name):
    return jax.named_scope(name) if CFG['scopes'] else _NoScope()


def _pieces(t, t1, ntc):
    pcs = []
    while t < t1:
        rb, c = divmod(t, ntc)
        n = min(t1 - t, ntc - c)
        pcs.append((rb, c, n))
        t += n
    return pcs


def _blocks(rb0, rb1, ntc, phase):
    lo, hi = rb0 * ntc, rb1 * ntc
    t = lo - ((lo - phase) % (2 * ST))
    out = []
    while t < hi:
        out.append([_pieces(max(t, lo), min(t + ST, hi), ntc),
                    _pieces(max(t + ST, lo), min(t + 2 * ST, hi), ntc)])
        t += 2 * ST
    sz = lambda b: sum(n for h in b for _, _, n in h)
    if len(out) > 2 and sz(out[0]) + sz(out[-1]) <= 2 * ST + 4:
        first, last = out.pop(0), out.pop()
        a, b = first[0] + first[1], last[0] + last[1]

        def join(p):
            q = []
            for x in p:
                if q and q[-1][0] == x[0] and q[-1][1] + q[-1][2] == x[1]:
                    q[-1] = (x[0], q[-1][1], q[-1][2] + x[2])
                else:
                    q.append(x)
            return q
        out.insert(0, [join(a), join(b)])
    return out


def _spread(streams):
    keyed = []
    for si, items in enumerate(streams):
        for i, x in enumerate(items):
            keyed.append(((i + (si + 1.0) / (len(streams) + 1)) / len(items), si, i, x))
    keyed.sort(key=lambda z: z[:3])
    return [z[3] for z in keyed]


def _deadline(streams):
    rem = [list(it) for it, _ in streams]
    total = sum(len(r) for r in rem)
    last_used = [-1] * len(streams)
    out = []
    for k in range(total):
        el = [s for s in range(len(streams)) if rem[s] and streams[s][1] <= k]
        if not el:
            el = [min((s for s in range(len(streams)) if rem[s]), key=lambda s: streams[s][1])]
        s = min(el, key=lambda s: (last_used[s], -len(rem[s])))
        last_used[s] = k
        out.append(rem[s].pop())
    return out[::-1]


def _layernorm(x, eps=1e-5):
    m = jnp.mean(x, axis=-1, keepdims=True)
    xc = x - m
    v = jnp.mean(xc * xc, axis=-1, keepdims=True)
    return xc * lax.rsqrt(v + eps)


def _dot(a, b):
    return jnp.dot(a, b, preferred_element_type=F32)


def _dot_nt(a, b):
    return lax.dot_general(a, b, (((1,), (1,)), ((), ())), preferred_element_type=F32)


def _kernel(x_hbm, k_hbm, v_hbm, wq_hbm, wo_hbm, wr_hbm, wg_hbm, wu_hbm, wd_hbm,
            c_hbm, wm_hbm, out_ref,
            x_v, c_v, wr_v, wm_v, wq_v, wo_v, wg_v, wu_v, wd_v, kbuf, vbuf,
            mod_s, h_s, q_s, s_s, p_s, l_s, o_s, acc_s, act_s, actb_s,
            sems, *, W):
    B, HKV, SK, _ = k_hbm.shape
    D = x_v.shape[1]
    FF = wg_v.shape[1]
    NRB = D // 8
    scale = DH ** -0.5
    S_SMALL, S_C, S_RING = 0, 3, 8
    LAG, WLAG = CFG['lag'], CFG['wlag']
    NKV = HKV * 2 * B * (W // 256)
    HS = NKV // HKV // GP

    def w_pairs(hbm, buf, tag, rb0, rb1, phase):
        def mk(pc):
            rb, c, n = pc
            idx = (pl.ds(rb * 8, 8), pl.ds(c * 128, n * 128))
            return lambda si: pltpu.make_async_copy(hbm.at[idx], buf.at[idx], sems.at[si])
        return [([mk(p) for p in f], [mk(p) for p in b], tag)
                for f, b in _blocks(rb0, rb1, buf.shape[1] // 128, phase)]

    PH = CFG['ph_kv']
    NJ = W // 256
    kv_geo = [((0, PH), (PH + 256 * (NJ - 1), 256 - PH))]
    kv_geo += [((PH + 256 * j, 128), (PH + 256 * j + 128, 128)) for j in range(NJ - 1)]

    def kv_copy(rnd, p, half):
        j, isv = p // 2, p % 2
        hbm, buf = ((k_hbm, kbuf), (v_hbm, vbuf))[isv]
        o, n = kv_geo[j][half]
        g = rnd // 8
        b = (j + isv * CFG['vb'] + (CFG['tb'] if j == 0 and half else 0) + 8 - rnd % 8) % 8
        return lambda si: pltpu.make_async_copy(
            hbm.at[b, g, pl.ds(SK - W + o, n), :], buf.at[g % 2, b, pl.ds(o, n), :], sems.at[si])

    RT = NRB - CFG['gu_tail']
    ns = CFG['nsub']

    def subs(hbm, buf, tag, rb1, phase):
        cuts = [rb1 * i // ns[tag] for i in range(ns[tag] + 1)]
        return [w_pairs(hbm, buf, tag, cuts[i], cuts[i + 1], phase) for i in range(ns[tag])]
    streams = (subs(wm_hbm, wm_v, 'M', NRB, CFG['ph_m']) + subs(wq_hbm, wq_v, 'Q', NRB, CFG['ph_q'])
               + subs(wo_hbm, wo_v, 'O', NRB, CFG['ph_q']) + subs(wg_hbm, wg_v, 'G', RT, CFG['ph_f'])
               + subs(wu_hbm, wu_v, 'U', RT, CFG['ph_f']))
    pairs_a = _spread(streams[0::2] + streams[1::2])

    fin = CFG['fin']
    d_rows = {'B%d' % k: (128 * k, 128 * (k + 1)) for k in range(4)}
    regions = sorted(d_rows, key=lambda nm: -fin[nm])

    def halves(pairs, key):
        n = CFG['tsub']
        return [(pairs[len(pairs) * i // n:len(pairs) * (i + 1) // n], fin[key]) for i in range(n)]
    streams = (halves(w_pairs(wg_hbm, wg_v, 'G', RT, NRB, CFG['ph_f']), 'G')
               + halves(w_pairs(wu_hbm, wu_v, 'U', RT, NRB, CFG['ph_f']), 'U'))
    for nm in regions:
        streams += halves(w_pairs(wd_hbm, wd_v, nm, d_rows[nm][0] // 8, d_rows[nm][1] // 8, CFG['ph_f']), nm)
    pairs_c = _deadline(streams)

    groups = []
    r = len(pairs_a) % GP
    if r:
        groups.append(pairs_a[:r])
    groups += [pairs_a[i:i + GP] for i in range(r, len(pairs_a), GP)]
    GA = len(groups)
    for n0 in range(0, NKV, GP):
        groups.append([([kv_copy(n // 16, n % 16, 0)], [kv_copy(n // 16, n % 16, 1)], 'KV')
                       for n in range(n0, n0 + GP)])
    GC = len(groups)
    last_of = {}
    cur = []
    for i, pr in enumerate(pairs_c):
        cur.append(pr)
        end_tag = all(q[2] != pr[2] for q in pairs_c[i + 1:])
        if len(cur) == GP or end_tag:
            if end_tag:
                last_of[pr[2]] = len(groups)
            groups.append(cur)
            cur = []
    NG = len(groups)
    d_cols = {}
    last = []
    c0 = 0
    for i, n in enumerate(CFG['c_split']):
        nm = 'C%d' % i
        d_rows[nm] = (512, D)
        d_cols[nm] = (c0, c0 + n * 128)
        for c in range(c0, c0 + n * 128, CFG['c_w']):
            idx = (pl.ds(512, D - 512), pl.ds(c, min(CFG['c_w'], c0 + n * 128 - c)))
            last.append((lambda si, idx=idx: pltpu.make_async_copy(wd_hbm.at[idx], wd_v.at[idx], sems.at[si]), S_C + i))
        regions.append(nm)
        c0 += n * 128
    assert c0 == FF

    bgs, at = [], {}
    for gi, grp in enumerate(groups):
        for k, (f, b, _) in enumerate(grp):
            at.setdefault(len(bgs) + LAG, []).append((gi, k == 0, f))
            bgs.extend((c, S_RING + gi % RS) for c in b)
    bgs.extend(last)
    steps = [[]]
    for i in range(max(len(bgs), max(at) + 1)):
        for gi, first, f in at.get(i, []):
            if first:
                steps.append([])
            steps[-1].extend((c, S_RING + gi % RS, FG) for c in f)
        if i < len(bgs):
            steps[-1].append(bgs[i] + (BG,))
    prime, steps = steps[0], steps[1:]
    assert len(steps) == NG

    def start(lst):
        for c, si, prio in lst:
            c(si).start(priority=prio)

    def wait_group(gi):
        for f, b, _ in groups[gi]:
            for c in f + b:
                c(S_RING + gi % RS).wait()

    owner, started = {}, {}
    gid = {}
    for gi, grp in enumerate(groups):
        for f, b, _ in grp:
            for c in f + b:
                gid[c] = gi
    for s in range(-1, NG + WLAG):
        if 0 <= s - WLAG:
            w = s - WLAG
            assert started.get(w, 0) == sum(len(f) + len(b) for f, b, _ in groups[w])
            owner.pop(w % RS, None)
        for c, si, _ in (prime if s < 0 else steps[s] if s < NG else []):
            if c in gid:
                assert owner.setdefault(gid[c] % RS, gid[c]) == gid[c]
                started[gid[c]] = started.get(gid[c], 0) + 1

    state = dict(issued=0, waited=0)

    def advance(n):
        for _ in range(n):
            if state['issued'] < NG:
                s = state['issued']
                while state['waited'] <= s - WLAG:
                    wait_group(state['waited']); state['waited'] += 1
                start(steps[s]); state['issued'] += 1

    def ensure(gi):
        while state['waited'] <= gi:
            if state['issued'] < min(NG, state['waited'] + WLAG + 1):
                advance(1)
            else:
                wait_group(state['waited']); state['waited'] += 1

    small = [pltpu.make_async_copy(c_hbm, c_v, sems.at[S_SMALL]),
             pltpu.make_async_copy(x_hbm, x_v, sems.at[S_SMALL + 1]),
             pltpu.make_async_copy(wr_hbm, wr_v, sems.at[S_SMALL + 2])]
    L0 = WLAG + WLAG % 2
    with scope('p0'):
        start(prime)
        for s in range(GA + L0):
            advance(1)
            if s == 0:
                for cp in small:
                    cp.start(priority=FG)
    for _ in range(CFG['pad']):
        pl.delay(1)

    row_s = lax.broadcasted_iota(jnp.int32, (2 * B, W), 0) % B
    row_o = lax.broadcasted_iota(jnp.int32, (2 * B, DH), 0) % B
    L1 = (NKV - LAG) // GP // 2 * 2

    def issue(rnd):
        for par in range(2):
            t = 2 * rnd + par
            rw, pw = rnd + (par - WLAG) // 2, (par - WLAG) % 2
            for p in range(pw * GP, (pw + 1) * GP):
                for half in range(2):
                    kv_copy(rw, p, half)(S_RING + (GA + t - WLAG) % RS).wait()
            for p in range(par * GP, (par + 1) * GP):
                kv_copy(rnd, p, 0)(S_RING + (GA + t) % RS).start(priority=FG)
                q = p + LAG
                kv_copy(rnd + q // 16, q % 16, 1)(
                    S_RING + (GA + 2 * rnd + q // GP) % RS).start(priority=BG)

    def qk(g, slot, bs):
        qh = q_s[g].astype(BF16)
        for b in bs:
            pltpu.store(s_s, _dot_nt(qh, kbuf[slot, b]), mask=row_s == b)

    def softmax():
        s = s_s[...]
        m = jnp.max(s, axis=-1, keepdims=True)
        e = jnp.exp((s - m) * scale)
        l_s[...] = jnp.broadcast_to(jnp.sum(e, axis=-1, keepdims=True), l_s.shape)
        p_s[...] = e.astype(BF16)

    def pv(slot, bs):
        pb = p_s[...]
        for b in bs:
            pltpu.store(o_s, _dot(pb, vbuf[slot, b]), mask=row_o == b)

    def project(g):
        o = (o_s[...] / l_s[...]).astype(BF16)
        o2 = jnp.concatenate([o[0:B], o[B:2 * B]], axis=1)
        col = g * (2 * DH)
        if not isinstance(g, int):
            col = pl.multiple_of(col, 2 * DH)
        acc_s[...] += _dot_nt(o2, wo_v[:, pl.ds(col, 2 * DH)])

    P0 = L0 // 2

    def body(it, carry):
        ph = it % 8
        g = it // 8 - 1
        slot = (g + 2) % 2

        @pl.when(it == P0)
        def _():
            for cp in small:
                cp.wait()
            c = c_v[...].astype(F32)
            sc = (c * jax.nn.sigmoid(c)).astype(BF16)
            mod = _dot(sc, wm_v[...])
            x = x_v[...].astype(F32)
            h_s[...] = _layernorm(x) * (1.0 + mod[:, D:2 * D]) + mod[:, 0:D]
            mod_s[...] = mod[:, 2 * D:6 * D]
            acc_s[...] = jnp.zeros_like(acc_s)

        @pl.when(it == P0 + 2)
        def _():
            q = _dot(h_s[...].astype(BF16), wq_v[...])
            for hq in range(HQ):
                q_s[hq // 2, (hq % 2) * B:(hq % 2 + 1) * B, :] = q[:, hq * DH:(hq + 1) * DH]

        @pl.when(g >= 0)
        def _():
            @pl.when(jnp.logical_or(ph == P0, ph == P0 + 1))
            def _():
                U = CFG['qk_unroll']
                b0 = (ph - P0) * (B // 2)
                lax.fori_loop(0, B // 2 // U,
                              lambda j, c: (qk(g, slot, [b0 + j * U + u for u in range(U)]), c)[1], 0)

            @pl.when(ph == P0 + CFG['sm_at'])
            def _():
                softmax()

            @pl.when(ph == P0 + CFG['pv_at'])
            def _():
                U = CFG['pv_unroll']
                lax.fori_loop(0, B // U,
                              lambda j, c: (pv(slot, [j * U + u for u in range(U)]), c)[1], 0)

            @pl.when(ph == P0 + 3)
            def _():
                project(g)

        with scope('issue'):
            issue(it)
        return carry

    assert P0 + 3 <= 5 and 2 * (P0 + CFG['pv_at']) * GP - 1 + LAG < HS * GP
    with scope('loop'):
        lax.fori_loop(L0 // 2, L1 // 2, body, 0)

    state.update(issued=GA + L1, waited=GA + L1 - WLAG)
    with scope('lastkv'):
        ensure(GC - 1)
    ta = list(CFG['tail_adv'])
    gl = HKV - 1
    for bs in CFG['tail_qk']:
        qk(gl, gl % 2, bs)
        advance(ta.pop(0))
    softmax()
    advance(ta.pop(0))
    for bs in CFG['tail_pv']:
        pv(gl % 2, bs)
        advance(ta.pop(0))
    project(gl)

    post = list(CFG['post'])

    mod = mod_s[...]
    ga, sb, cb, gb = (mod[:, i * D:(i + 1) * D] for i in range(4))
    x2 = x_v[...].astype(F32) + ga * acc_s[...]
    h2 = _layernorm(x2) * (1.0 + cb) + sb
    h2b = h2.astype(BF16)
    wr = wr_v[...].astype(F32).reshape(1, D)
    rsel = jax.nn.sigmoid(jnp.sum(h2 * wr, axis=-1, keepdims=True))
    acc_s[...] = x2 + gb * h2
    h_s[...] = gb * rsel
    with scope('waitg'):
        advance(post.pop(0))
        ensure(last_of['G'])
    g = _dot(h2b, wg_v[...])
    act_s[...] = g * jax.nn.sigmoid(g)
    with scope('waitu'):
        advance(post.pop(0))
        ensure(last_of['U'])
    u = _dot(h2b, wu_v[...])
    actb_s[...] = (act_s[...] * u).astype(BF16)
    for nm in regions:
        r0, r1 = d_rows[nm]
        f0, f1 = d_cols.get(nm, (0, FF))
        with scope('wait' + nm):
            advance(post.pop(0) if post else 0)
            if nm in last_of:
                ensure(last_of[nm])
            else:
                ensure(NG - 1)
                blk = wd_v.at[pl.ds(r0, r1 - r0), pl.ds(f0, f1 - f0)]
                pltpu.make_async_copy(blk, blk, sems.at[S_C + int(nm[1])]).wait()
        y = _dot_nt(actb_s[:, f0:f1], wd_v[r0:r1, f0:f1])
        val = acc_s[:, r0:r1] + h_s[:, r0:r1] * y
        if f1 < FF:
            acc_s[:, r0:r1] = val
        else:
            out_ref[:, r0:r1] = val.astype(out_ref.dtype)
    assert state['issued'] == NG and state['waited'] == NG


@jax.jit
def pallas_adaLN_cond__sliding_block_cached__moe_arch_mod__decode_kernel(
    A_x, A_k_cache, A_v_cache, A_wq, A_wo, B_x, B_w_r, B_w_gate, B_w_up, B_w_down, c, w_mod):
    B, SQ, D = A_x.shape
    _, HKV, SK, _ = A_k_cache.shape
    FF = B_w_gate.shape[1]
    W = min(4096, max(256, SK // 4))
    assert SQ == 1 and HQ == 2 * HKV and B == 8

    vm = pltpu.VMEM
    scratch = [
        vm((B, D), BF16), vm((B, D), BF16), vm((D,), BF16),
        vm((D, 6 * D), BF16), vm((D, HQ * DH), BF16), vm((D, HQ * DH), BF16),
        vm((D, FF), BF16), vm((D, FF), BF16), vm((D, FF), BF16),
        vm((2, B, W, DH), BF16), vm((2, B, W, DH), BF16),
        vm((B, 4 * D), F32),
        vm((B, D), F32),
        vm((HKV, 2 * B, DH), F32),
        vm((2 * B, W), F32),
        vm((2 * B, W), BF16),
        vm((2 * B, DH), F32),
        vm((2 * B, DH), F32),
        vm((B, D), F32),
        vm((B, FF), F32),
        vm((B, FF), BF16),
        pltpu.SemaphoreType.DMA((8 + RS,)),
    ]
    out = pl.pallas_call(
        functools.partial(_kernel, W=W),
        out_shape=jax.ShapeDtypeStruct((B, D), A_x.dtype),
        in_specs=[pl.BlockSpec(memory_space=pl.ANY)] * 11,
        out_specs=pl.BlockSpec(memory_space=pltpu.VMEM),
        scratch_shapes=scratch,
        compiler_params=pltpu.CompilerParams(
            vmem_limit_bytes=64 * 1024 * 1024,
            disable_bounds_checks=True,
            disable_semaphore_checks=True,
        ),
    )(A_x.reshape(B, D), A_k_cache, A_v_cache, A_wq, A_wo.T, B_w_r,
      B_w_gate, B_w_up, B_w_down.T, c, w_mod)
    return out.reshape(B, SQ, D)
```

```python
import functools

import jax
import jax.numpy as jnp
from jax import lax
import jax.experimental.pallas as pl
import jax.experimental.pallas.tpu as pltpu

F32 = jnp.float32
BF16 = jnp.bfloat16

HQ = 32
DH = 128
FG, BG = 0, 1
ST = 16
GP = 8
RS = 16

CFG = dict(scopes=False, ph_kv=144, ph_q=18, ph_f=24, ph_m=21, lag=26, wlag=4,
           gu_tail=16, sp=8, vb=4, tb=4,
           fin=dict(G=64, U=52, B0=24, B1=16, B2=8, B3=0), tsub=2,
           c_split=(24, 12), c_w=128, pad=0,
           l_qk=((0, 1), (2, 3), (4, 5), (6, 7)), l_pv=((0, 1, 2, 3), (4, 5, 6, 7)), tail_qk=((0, 1, 2, 3), (4, 5, 6, 7)), tail_pv=((0, 1, 2, 3, 4, 5, 6, 7),), tail_adv=(1, 0, 2, 1),
           post=(1, 2, 2, 1, 1, 1, 1, 1))


class _NoScope:
    def __enter__(self): return self
    def __exit__(self, *a): return False


def scope(name):
    return jax.named_scope(name) if CFG['scopes'] else _NoScope()


def _pieces(t, t1, ntc):
    pcs = []
    while t < t1:
        rb, c = divmod(t, ntc)
        n = min(t1 - t, ntc - c)
        pcs.append((rb, c, n))
        t += n
    return pcs


def _blocks(rb0, rb1, ntc, phase):
    lo, hi = rb0 * ntc, rb1 * ntc
    t = lo - ((lo - phase) % (2 * ST))
    out = []
    while t < hi:
        out.append([_pieces(max(t, lo), min(t + ST, hi), ntc),
                    _pieces(max(t + ST, lo), min(t + 2 * ST, hi), ntc)])
        t += 2 * ST
    sz = lambda b: sum(n for h in b for _, _, n in h)
    if len(out) > 2 and sz(out[0]) + sz(out[-1]) <= 2 * ST + 4:
        first, last = out.pop(0), out.pop()
        a, b = first[0] + first[1], last[0] + last[1]

        def join(p):
            q = []
            for x in p:
                if q and q[-1][0] == x[0] and q[-1][1] + q[-1][2] == x[1]:
                    q[-1] = (x[0], q[-1][1], q[-1][2] + x[2])
                else:
                    q.append(x)
            return q
        out.insert(0, [join(a), join(b)])
    return out


def _spread(streams):
    keyed = []
    for si, items in enumerate(streams):
        for i, x in enumerate(items):
            keyed.append(((i + (si + 1.0) / (len(streams) + 1)) / len(items), si, i, x))
    keyed.sort(key=lambda z: z[:3])
    return [z[3] for z in keyed]


def _deadline(streams):
    rem = [list(it) for it, _ in streams]
    total = sum(len(r) for r in rem)
    last_used = [-1] * len(streams)
    out = []
    for k in range(total):
        el = [s for s in range(len(streams)) if rem[s] and streams[s][1] <= k]
        if not el:
            el = [min((s for s in range(len(streams)) if rem[s]), key=lambda s: streams[s][1])]
        s = min(el, key=lambda s: (last_used[s], -len(rem[s])))
        last_used[s] = k
        out.append(rem[s].pop())
    return out[::-1]


def _layernorm(x, eps=1e-5):
    m = jnp.mean(x, axis=-1, keepdims=True)
    xc = x - m
    v = jnp.mean(xc * xc, axis=-1, keepdims=True)
    return xc * lax.rsqrt(v + eps)


def _dot(a, b):
    return jnp.dot(a, b, preferred_element_type=F32)


def _dot_nt(a, b):
    return lax.dot_general(a, b, (((1,), (1,)), ((), ())), preferred_element_type=F32)


def _kernel(x_hbm, k_hbm, v_hbm, wq_hbm, wo_hbm, wr_hbm, wg_hbm, wu_hbm, wd_hbm,
            c_hbm, wm_hbm, out_ref,
            x_v, c_v, wr_v, wm_v, wq_v, wo_v, wg_v, wu_v, wd_v, kbuf, vbuf,
            mod_s, h_s, q_s, s_s, p_s, l_s, o_s, acc_s, act_s, actb_s,
            sems, *, W):
    B, HKV, SK, _ = k_hbm.shape
    D = x_v.shape[1]
    FF = wg_v.shape[1]
    NRB = D // 8
    scale = DH ** -0.5
    S_SMALL, S_C, S_RING = 0, 3, 8
    LAG, WLAG = CFG['lag'], CFG['wlag']
    NKV = HKV * 2 * B * (W // 256)
    HS = NKV // HKV // GP

    def w_pairs(hbm, buf, tag, rb0, rb1, phase):
        def mk(pc):
            rb, c, n = pc
            idx = (pl.ds(rb * 8, 8), pl.ds(c * 128, n * 128))
            return lambda si: pltpu.make_async_copy(hbm.at[idx], buf.at[idx], sems.at[si])
        return [([mk(p) for p in f], [mk(p) for p in b], tag)
                for f, b in _blocks(rb0, rb1, buf.shape[1] // 128, phase)]

    PH = CFG['ph_kv']
    NJ = W // 256
    kv_geo = [((0, PH), (PH + 256 * (NJ - 1), 256 - PH))]
    kv_geo += [((PH + 256 * j, 128), (PH + 256 * j + 128, 128)) for j in range(NJ - 1)]

    def kv_copy(rnd, p, half, g):
        j, isv = p // 2, p % 2
        hbm, buf = ((k_hbm, kbuf), (v_hbm, vbuf))[isv]
        o, n = kv_geo[j][half]
        b = (j + isv * CFG['vb'] + (CFG['tb'] if j == 0 and half else 0) - rnd) % 8
        return lambda si: pltpu.make_async_copy(
            hbm.at[b, g, pl.ds(SK - W + o, n), :], buf.at[g % 2, b, pl.ds(o, n), :], sems.at[si])

    RT = NRB - CFG['gu_tail']
    streams = []
    for hbm, buf, tag, rb1, phase in ((wm_hbm, wm_v, 'M', NRB, CFG['ph_m']), (wq_hbm, wq_v, 'Q', NRB, CFG['ph_q']),
                                      (wo_hbm, wo_v, 'O', NRB, CFG['ph_q']), (wg_hbm, wg_v, 'G', RT, CFG['ph_f']),
                                      (wu_hbm, wu_v, 'U', RT, CFG['ph_f'])):
        prs = w_pairs(hbm, buf, tag, 0, rb1, phase)
        streams += [prs[i:i + CFG['sp']] for i in range(0, len(prs), CFG['sp'])]
    pairs_a = _spread(streams)

    fin = CFG['fin']
    d_rows = {'B%d' % k: (128 * k, 128 * (k + 1)) for k in range(4)}
    regions = sorted(d_rows, key=lambda nm: -fin[nm])

    def halves(pairs, key):
        n = CFG['tsub']
        return [(pairs[len(pairs) * i // n:len(pairs) * (i + 1) // n], fin[key]) for i in range(n)]
    streams = (halves(w_pairs(wg_hbm, wg_v, 'G', RT, NRB, CFG['ph_f']), 'G')
               + halves(w_pairs(wu_hbm, wu_v, 'U', RT, NRB, CFG['ph_f']), 'U'))
    for nm in regions:
        streams += halves(w_pairs(wd_hbm, wd_v, nm, d_rows[nm][0] // 8, d_rows[nm][1] // 8, CFG['ph_f']), nm)
    pairs_c = _deadline(streams)

    groups = []
    r = len(pairs_a) % GP
    if r:
        groups.append(pairs_a[:r])
    groups += [pairs_a[i:i + GP] for i in range(r, len(pairs_a), GP)]
    GA = len(groups)
    for n0 in range(0, NKV, GP):
        groups.append([([kv_copy(n // 16 % 8, n % 16, 0, n // 128)], [kv_copy(n // 16 % 8, n % 16, 1, n // 128)], 'KV')
                       for n in range(n0, n0 + GP)])
    GC = len(groups)
    last_of = {}
    cur = []
    for i, pr in enumerate(pairs_c):
        cur.append(pr)
        end_tag = all(q[2] != pr[2] for q in pairs_c[i + 1:])
        if len(cur) == GP or end_tag:
            if end_tag:
                last_of[pr[2]] = len(groups)
            groups.append(cur)
            cur = []
    NG = len(groups)
    d_cols = {}
    last = []
    c0 = 0
    for i, n in enumerate(CFG['c_split']):
        nm = 'C%d' % i
        d_rows[nm] = (512, D)
        d_cols[nm] = (c0, c0 + n * 128)
        for c in range(c0, c0 + n * 128, CFG['c_w']):
            idx = (pl.ds(512, D - 512), pl.ds(c, min(CFG['c_w'], c0 + n * 128 - c)))
            last.append((lambda si, idx=idx: pltpu.make_async_copy(wd_hbm.at[idx], wd_v.at[idx], sems.at[si]), S_C + i))
        regions.append(nm)
        c0 += n * 128
    assert c0 == FF

    bgs, at = [], {}
    for gi, grp in enumerate(groups):
        for k, (f, b, _) in enumerate(grp):
            at.setdefault(len(bgs) + LAG, []).append((gi, k == 0, f))
            bgs.extend((c, S_RING + gi % RS) for c in b)
    bgs.extend(last)
    steps = [[]]
    for i in range(max(len(bgs), max(at) + 1)):
        for gi, first, f in at.get(i, []):
            if first:
                steps.append([])
            steps[-1].extend((c, S_RING + gi % RS, FG) for c in f)
        if i < len(bgs):
            steps[-1].append(bgs[i] + (BG,))
    prime, steps = steps[0], steps[1:]
    assert len(steps) == NG

    def start(lst):
        for c, si, prio in lst:
            c(si).start(priority=prio)

    def wait_group(gi):
        for f, b, _ in groups[gi]:
            for c in f + b:
                c(S_RING + gi % RS).wait()

    owner, started = {}, {}
    gid = {}
    for gi, grp in enumerate(groups):
        for f, b, _ in grp:
            for c in f + b:
                gid[c] = gi
    for s in range(-1, NG + WLAG):
        if 0 <= s - WLAG:
            w = s - WLAG
            assert started.get(w, 0) == sum(len(f) + len(b) for f, b, _ in groups[w])
            owner.pop(w % RS, None)
        for c, si, _ in (prime if s < 0 else steps[s] if s < NG else []):
            if c in gid:
                assert owner.setdefault(gid[c] % RS, gid[c]) == gid[c]
                started[gid[c]] = started.get(gid[c], 0) + 1

    state = dict(issued=0, waited=0)

    def advance(n):
        for _ in range(n):
            if state['issued'] < NG:
                s = state['issued']
                while state['waited'] <= s - WLAG:
                    wait_group(state['waited']); state['waited'] += 1
                start(steps[s]); state['issued'] += 1

    def ensure(gi):
        while state['waited'] <= gi:
            if state['issued'] < min(NG, state['waited'] + WLAG + 1):
                advance(1)
            else:
                wait_group(state['waited']); state['waited'] += 1

    row_s = lax.broadcasted_iota(jnp.int32, (2 * B, W), 0) % B
    row_o = lax.broadcasted_iota(jnp.int32, (2 * B, DH), 0) % B

    def qk(g, slot, bs):
        qh = q_s[g].astype(BF16)
        for b in bs:
            pltpu.store(s_s, _dot_nt(qh, kbuf[slot, b]), mask=row_s == b)

    def softmax():
        s = s_s[...]
        m = jnp.max(s, axis=-1, keepdims=True)
        e = jnp.exp((s - m) * scale)
        l_s[...] = jnp.broadcast_to(jnp.sum(e, axis=-1, keepdims=True), l_s.shape)
        p_s[...] = e.astype(BF16)

    def pv(slot, bs):
        pb = p_s[...]
        for b in bs:
            pltpu.store(o_s, _dot(pb, vbuf[slot, b]), mask=row_o == b)

    def project(g):
        o = (o_s[...] / l_s[...]).astype(BF16)
        o2 = jnp.concatenate([o[0:B], o[B:2 * B]], axis=1)
        col = g * (2 * DH)
        if not isinstance(g, int):
            col = pl.multiple_of(col, 2 * DH)
        acc_s[...] += _dot_nt(o2, wo_v[:, pl.ds(col, 2 * DH)])

    small = [pltpu.make_async_copy(c_hbm, c_v, sems.at[S_SMALL]),
             pltpu.make_async_copy(x_hbm, x_v, sems.at[S_SMALL + 1]),
             pltpu.make_async_copy(wr_hbm, wr_v, sems.at[S_SMALL + 2])]
    L1 = (NKV - LAG) // GP
    L0 = L1 - (HKV - 1) * HS
    with scope('p0'):
        start(prime)
        advance(1)
        for cp in small:
            cp.start(priority=FG)
        advance(GA + WLAG - 1)
    assert state['waited'] >= GA
    for cp in small:
        cp.wait()
    c = c_v[...].astype(F32)
    sc = (c * jax.nn.sigmoid(c)).astype(BF16)
    mod = _dot(sc, wm_v[:, 0:2 * D])
    x = x_v[...].astype(F32)
    h_s[...] = _layernorm(x) * (1.0 + mod[:, D:2 * D]) + mod[:, 0:D]
    advance(1)
    mod_s[...] = _dot(sc, wm_v[:, 2 * D:6 * D])
    acc_s[...] = jnp.zeros_like(acc_s)
    advance(1)
    hb = h_s[...].astype(BF16)
    for part in range(2):
        q = _dot(hb, wq_v[:, part * HKV * DH:(part + 1) * HKV * DH])
        for hq in range(HKV):
            q_s[part * (HKV // 2) + hq // 2, (hq % 2) * B:(hq % 2 + 1) * B, :] = q[:, hq * DH:(hq + 1) * DH]
        advance(1)
    advance(GA + L0 - state['issued'])
    for _ in range(CFG['pad']):
        pl.delay(1)

    K0 = HS - 1 + WLAG - L0

    def body(g, carry):
        slot = g % 2
        work = [functools.partial(qk, g, slot, bs) for bs in CFG['l_qk']] + [softmax]
        work += [functools.partial(pv, slot, bs) for bs in CFG['l_pv']] + [functools.partial(project, g)]
        assert K0 + len(work) <= HS
        for k in range(HS):
            t = L0 + k

            def cp(n, half):
                return kv_copy(n // 16 % 8, n % 16, half, g + n // (HS * GP))(S_RING + (GA + n // GP) % RS)
            for n in range((t - WLAG) * GP, (t - WLAG + 1) * GP):
                cp(n, 0).wait()
                cp(n, 1).wait()
            for n in range(t * GP, (t + 1) * GP):
                cp(n, 0).start(priority=FG)
                cp(n + LAG, 1).start(priority=BG)
            if K0 <= k < K0 + len(work):
                work[k - K0]()
        return carry

    assert HS % RS == 0 and (L0 + HS) * GP - 1 + LAG < 2 * HS * GP
    with scope('loop'):
        lax.fori_loop(0, HKV - 1, body, 0)

    state.update(issued=GA + L1, waited=GA + L1 - WLAG)
    with scope('lastkv'):
        ensure(GC - 1)
    ta = list(CFG['tail_adv'])
    gl = HKV - 1
    for bs in CFG['tail_qk']:
        qk(gl, gl % 2, bs)
        advance(ta.pop(0))
    softmax()
    advance(ta.pop(0))
    for bs in CFG['tail_pv']:
        pv(gl % 2, bs)
        advance(ta.pop(0))
    project(gl)

    post = list(CFG['post'])

    mod = mod_s[...]
    ga, sb, cb, gb = (mod[:, i * D:(i + 1) * D] for i in range(4))
    x2 = x_v[...].astype(F32) + ga * acc_s[...]
    h2 = _layernorm(x2) * (1.0 + cb) + sb
    h2b = h2.astype(BF16)
    wr = wr_v[...].astype(F32).reshape(1, D)
    rsel = jax.nn.sigmoid(jnp.sum(h2 * wr, axis=-1, keepdims=True))
    acc_s[...] = x2 + gb * h2
    h_s[...] = gb * rsel
    with scope('waitg'):
        advance(post.pop(0))
        ensure(last_of['G'])
    g = _dot(h2b, wg_v[...])
    act_s[...] = g * jax.nn.sigmoid(g)
    with scope('waitu'):
        advance(post.pop(0))
        ensure(last_of['U'])
    u = _dot(h2b, wu_v[...])
    actb_s[...] = (act_s[...] * u).astype(BF16)
    for nm in regions:
        r0, r1 = d_rows[nm]
        f0, f1 = d_cols.get(nm, (0, FF))
        with scope('wait' + nm):
            advance(post.pop(0) if post else 0)
            if nm in last_of:
                ensure(last_of[nm])
            else:
                ensure(NG - 1)
                blk = wd_v.at[pl.ds(r0, r1 - r0), pl.ds(f0, f1 - f0)]
                pltpu.make_async_copy(blk, blk, sems.at[S_C + int(nm[1])]).wait()
        y = _dot_nt(actb_s[:, f0:f1], wd_v[r0:r1, f0:f1])
        val = acc_s[:, r0:r1] + h_s[:, r0:r1] * y
        if f1 < FF:
            acc_s[:, r0:r1] = val
        else:
            out_ref[:, r0:r1] = val.astype(out_ref.dtype)
    assert state['issued'] == NG and state['waited'] == NG


@jax.jit
def pallas_adaLN_cond__sliding_block_cached__moe_arch_mod__decode_kernel(
    A_x, A_k_cache, A_v_cache, A_wq, A_wo, B_x, B_w_r, B_w_gate, B_w_up, B_w_down, c, w_mod):
    B, SQ, D = A_x.shape
    _, HKV, SK, _ = A_k_cache.shape
    FF = B_w_gate.shape[1]
    W = min(4096, max(256, SK // 4))
    assert SQ == 1 and HQ == 2 * HKV and B == 8

    vm = pltpu.VMEM
    scratch = [
        vm((B, D), BF16), vm((B, D), BF16), vm((D,), BF16),
        vm((D, 6 * D), BF16), vm((D, HQ * DH), BF16), vm((D, HQ * DH), BF16),
        vm((D, FF), BF16), vm((D, FF), BF16), vm((D, FF), BF16),
        vm((2, B, W, DH), BF16), vm((2, B, W, DH), BF16),
        vm((B, 4 * D), F32),
        vm((B, D), F32),
        vm((HKV, 2 * B, DH), F32),
        vm((2 * B, W), F32),
        vm((2 * B, W), BF16),
        vm((2 * B, DH), F32),
        vm((2 * B, DH), F32),
        vm((B, D), F32),
        vm((B, FF), F32),
        vm((B, FF), BF16),
        pltpu.SemaphoreType.DMA((8 + RS,)),
    ]
    out = pl.pallas_call(
        functools.partial(_kernel, W=W),
        out_shape=jax.ShapeDtypeStruct((B, D), A_x.dtype),
        in_specs=[pl.BlockSpec(memory_space=pl.ANY)] * 11,
        out_specs=pl.BlockSpec(memory_space=pltpu.VMEM),
        scratch_shapes=scratch,
        compiler_params=pltpu.CompilerParams(
            vmem_limit_bytes=64 * 1024 * 1024,
            disable_bounds_checks=True,
            disable_semaphore_checks=True,
        ),
    )(A_x.reshape(B, D), A_k_cache, A_v_cache, A_wq, A_wo.T, B_w_r,
      B_w_gate, B_w_up, B_w_down.T, c, w_mod)
    return out.reshape(B, SQ, D)
```

```python
import functools

import jax
import jax.numpy as jnp
from jax import lax
import jax.experimental.pallas as pl
import jax.experimental.pallas.tpu as pltpu

F32 = jnp.float32
BF16 = jnp.bfloat16

HQ = 32
DH = 128
FG, BG = 0, 1
HALF = 16
GP = 8
RS = 16
LAG = 26
WLAG = 4
PH_KV = 144
PH_Q, PH_F, PH_M = 18, 24, 21
TAIL_RB = 16
TAIL_END = dict(G=64, U=52, B3=24, B1=16, B2=8, B0=0)
LAST_COLS = (24, 12)
S_SMALL, S_LAST, S_RING = 0, 3, 5


def _pieces(t, t1, ntc):
    pcs = []
    while t < t1:
        rb, c = divmod(t, ntc)
        n = min(t1 - t, ntc - c)
        pcs.append((rb, c, n))
        t += n
    return pcs


def _blocks(rb0, rb1, ntc, phase):
    lo, hi = rb0 * ntc, rb1 * ntc
    first = lo + (phase - lo) % (2 * HALF)
    last = hi - (hi - phase) % (2 * HALF)
    out = [(_pieces(lo, first, ntc), _pieces(last, hi, ntc))]
    for t in range(first, last, 2 * HALF):
        out.append((_pieces(t, t + HALF, ntc), _pieces(t + HALF, t + 2 * HALF, ntc)))
    return out


def _spread(streams):
    keyed = [((i + (s + 1.0) / (len(streams) + 1)) / len(items), s, i)
             for s, items in enumerate(streams) for i in range(len(items))]
    return [streams[s][i] for _, s, i in sorted(keyed)]


def _deadline(streams):
    rem = [list(items) for items, _ in streams]
    used = [-1] * len(streams)
    out = []
    for k in range(sum(len(r) for r in rem)):
        ok = [s for s in range(len(streams)) if rem[s] and streams[s][1] <= k]
        s = min(ok, key=lambda s: (used[s], -len(rem[s])))
        used[s] = k
        out.append(rem[s].pop())
    return out[::-1]


def _layernorm(x, eps=1e-5):
    m = jnp.mean(x, axis=-1, keepdims=True)
    xc = x - m
    v = jnp.mean(xc * xc, axis=-1, keepdims=True)
    return xc * lax.rsqrt(v + eps)


def _dot(a, b):
    return jnp.dot(a, b, preferred_element_type=F32)


def _dot_nt(a, b):
    return lax.dot_general(a, b, (((1,), (1,)), ((), ())), preferred_element_type=F32)


def _kernel(x_hbm, k_hbm, v_hbm, wq_hbm, wo_hbm, wr_hbm, wg_hbm, wu_hbm, wd_hbm,
            c_hbm, wm_hbm, out_hbm,
            x_v, c_v, wr_v, wm_v, wq_v, wo_v, wg_v, wu_v, wd_v, kbuf, vbuf,
            mod_s, h_s, q_s, s_s, p_s, l_s, o_s, acc_s, act_s, actb_s, out_v,
            sems):
    B, HKV, SK, _ = k_hbm.shape
    W = kbuf.shape[2]
    D = x_v.shape[1]
    FF = wg_v.shape[1]
    NRB = D // 8
    NJ = W // 256
    HB = 2 * B * NJ
    HS = HB // GP
    NKV = HKV * HB
    DL = D // 128 * 128

    def rect(hbm, buf, r0, nr, c0, nc):
        idx = (pl.ds(r0, nr), pl.ds(c0, nc))
        return lambda si: pltpu.make_async_copy(hbm.at[idx], buf.at[idx], sems.at[si])

    def w_blocks(hbm, buf, tag, rb0, rb1, phase):
        mk = lambda pcs: [rect(hbm, buf, rb * 8, 8, c * 128, n * 128) for rb, c, n in pcs]
        return [(mk(f), mk(b), tag) for f, b in _blocks(rb0, rb1, buf.shape[1] // 128, phase)]

    kv_rows = [((0, PH_KV), (PH_KV + 256 * (NJ - 1), 256 - PH_KV))]
    kv_rows += [((PH_KV + 256 * j, 128), (PH_KV + 256 * j + 128, 128)) for j in range(NJ - 1)]

    def kv_copy(g, n, half):
        rnd, j, isv = n // (2 * NJ), n // 2 % NJ, n % 2
        hbm, buf = ((k_hbm, kbuf), (v_hbm, vbuf))[isv]
        o, rows = kv_rows[j][half]
        b = (j - rnd + (B // 2) * (isv + (j == 0 and half == 1))) % B
        return lambda si: pltpu.make_async_copy(
            hbm.at[b, g, pl.ds(SK - W + o, rows), :],
            buf.at[g % 2, b, pl.ds(o, rows), :], sems.at[si])

    RT = NRB - TAIL_RB
    streams = []
    for hbm, buf, rb1, phase in ((wm_hbm, wm_v, NRB, PH_M), (wq_hbm, wq_v, NRB, PH_Q),
                                 (wo_hbm, wo_v, NRB, PH_Q), (wg_hbm, wg_v, RT, PH_F),
                                 (wu_hbm, wu_v, RT, PH_F)):
        blks = w_blocks(hbm, buf, 'W', 0, rb1, phase)
        streams += [blks[i:i + 8] for i in range(0, len(blks), 8)]
    head = _spread(streams)

    pieces = {'B%d' % k: (128 * k, 128 * (k + 1), 0, FF) for k in range(DL // 128)}
    order = sorted(pieces, key=lambda nm: -TAIL_END[nm])
    streams = []
    for hbm, buf, tag, rb0, rb1 in (
            [(wg_hbm, wg_v, 'G', RT, NRB), (wu_hbm, wu_v, 'U', RT, NRB)]
            + [(wd_hbm, wd_v, nm, pieces[nm][0] // 8, pieces[nm][1] // 8) for nm in order]):
        blks = w_blocks(hbm, buf, tag, rb0, rb1, PH_F)
        streams += [(blks[:len(blks) // 2], TAIL_END[tag]), (blks[len(blks) // 2:], TAIL_END[tag])]
    tail = _deadline(streams)

    last = []
    c0 = 0
    for i, n in enumerate(LAST_COLS):
        pieces['C%d' % i] = (DL, D, c0, c0 + n * 128)
        order.append('C%d' % i)
        last += [(rect(wd_hbm, wd_v, DL, D - DL, c, 128), S_LAST + i)
                 for c in range(c0, c0 + n * 128, 128)]
        c0 += n * 128
    assert c0 == FF

    r = len(head) % GP
    groups = [head[:r]] * (r > 0) + [head[i:i + GP] for i in range(r, len(head), GP)]
    GA = len(groups)
    groups += [[([kv_copy(n // HB, n % HB, 0)], [kv_copy(n // HB, n % HB, 1)], 'KV')
                for n in range(n0, n0 + GP)] for n0 in range(0, NKV, GP)]
    GC = len(groups)
    last_of = {}
    cur = []
    for i, blk in enumerate(tail):
        cur.append(blk)
        done = all(nxt[2] != blk[2] for nxt in tail[i + 1:])
        if done:
            last_of[blk[2]] = len(groups)
        if done or len(cur) == GP:
            groups.append(cur)
            cur = []
    NG = len(groups)
    sem_of = lambda gi: S_RING + gi % RS

    bgs, fg_at = [], {}
    for gi, grp in enumerate(groups):
        for k, (f, b, _) in enumerate(grp):
            fg_at.setdefault(len(bgs) + LAG, []).append((gi, k == 0, f))
            bgs += [(c, sem_of(gi)) for c in b]
    bgs += last
    steps = [[]]
    for i in range(max(len(bgs), max(fg_at) + 1)):
        for gi, first, f in fg_at.get(i, []):
            if first:
                steps.append([])
            steps[-1] += [(c, sem_of(gi), FG) for c in f]
        if i < len(bgs):
            steps[-1].append(bgs[i] + (BG,))
    prime, steps = steps[0], steps[1:]
    assert len(steps) == NG

    group_of = {c: gi for gi, grp in enumerate(groups) for f, b, _ in grp for c in f + b}
    owner, started = {}, [0] * NG
    for s in range(-1, NG + WLAG):
        if s >= WLAG:
            assert started[s - WLAG] == sum(len(f) + len(b) for f, b, _ in groups[s - WLAG])
            del owner[sem_of(s - WLAG)]
        for c, si, _ in (prime if s < 0 else steps[s] if s < NG else []):
            if c in group_of:
                assert owner.setdefault(si, group_of[c]) == group_of[c]
                started[group_of[c]] += 1

    state = dict(issued=0, waited=0)

    def start(lst):
        for c, si, prio in lst:
            c(si).start(priority=prio)

    def wait_next():
        gi = state['waited']
        for f, b, _ in groups[gi]:
            for c in f + b:
                c(sem_of(gi)).wait()
        state['waited'] += 1

    def advance(n):
        for _ in range(min(n, NG - state['issued'])):
            while state['waited'] <= state['issued'] - WLAG:
                wait_next()
            start(steps[state['issued']])
            state['issued'] += 1

    def ensure(gi):
        while state['waited'] <= gi:
            if state['issued'] < min(NG, state['waited'] + WLAG + 1):
                advance(1)
            else:
                wait_next()

    row_s = lax.broadcasted_iota(jnp.int32, (2 * B, W), 0) % B
    row_o = lax.broadcasted_iota(jnp.int32, (2 * B, DH), 0) % B

    def scores(g, bs):
        qh = q_s[g].astype(BF16)
        for b in bs:
            pltpu.store(s_s, _dot_nt(qh, kbuf[g % 2, b]), mask=row_s == b)

    def softmax():
        s = s_s[...]
        m = jnp.max(s, axis=-1, keepdims=True)
        e = jnp.exp((s - m) * DH ** -0.5)
        l_s[...] = jnp.broadcast_to(jnp.sum(e, axis=-1, keepdims=True), l_s.shape)
        p_s[...] = e.astype(BF16)

    def values(g, bs):
        p = p_s[...]
        for b in bs:
            pltpu.store(o_s, _dot(p, vbuf[g % 2, b]), mask=row_o == b)

    def project(g):
        o = (o_s[...] / l_s[...]).astype(BF16)
        o = jnp.concatenate([o[0:B], o[B:2 * B]], axis=1)
        col = g * (2 * DH)
        if not isinstance(g, int):
            col = pl.multiple_of(col, 2 * DH)
        acc_s[...] += _dot_nt(o, wo_v[:, pl.ds(col, 2 * DH)])

    small = [pltpu.make_async_copy(src, dst, sems.at[S_SMALL + i])
             for i, (src, dst) in enumerate(((c_hbm, c_v), (x_hbm, x_v), (wr_hbm, wr_v)))]
    start(prime)
    advance(1)
    for cp in small:
        cp.start(priority=FG)
    ensure(GA - 1)
    for cp in small:
        cp.wait()
    c = c_v[...].astype(F32)
    sc = (c * jax.nn.sigmoid(c)).astype(BF16)
    mod = _dot(sc, wm_v[:, 0:2 * D])
    h_s[...] = _layernorm(x_v[...].astype(F32)) * (1.0 + mod[:, D:2 * D]) + mod[:, 0:D]
    advance(1)
    mod_s[...] = _dot(sc, wm_v[:, 2 * D:6 * D])
    acc_s[...] = jnp.zeros_like(acc_s)
    s_s[...] = jnp.zeros_like(s_s)
    o_s[...] = jnp.zeros_like(o_s)
    advance(1)
    hb = h_s[...].astype(BF16)
    for part in range(2):
        q = _dot(hb, wq_v[:, part * HKV * DH:(part + 1) * HKV * DH])
        for i in range(HKV):
            q_s[(part * HKV + i) // 2, (i % 2) * B:(i % 2 + 1) * B, :] = q[:, i * DH:(i + 1) * DH]
        advance(1)

    L1 = (NKV - LAG) // GP
    L0 = L1 - (HKV - 1) * HS
    K0 = HS - 1 + WLAG - L0
    advance(GA + L0 - state['issued'])
    assert HS % RS == 0 and L0 >= WLAG and (L0 + HS) * GP + LAG <= 2 * HB

    def body(g, carry):
        work = [functools.partial(scores, g, (b, b + 1)) for b in range(0, B, 2)] + [softmax]
        work += [functools.partial(values, g, range(b, b + 4)) for b in range(0, B, 4)]
        work += [functools.partial(project, g)]
        assert K0 + len(work) <= HS
        copy = lambda n, half: kv_copy(g + n // HB, n % HB, half)(sem_of(GA + n // GP))
        for k in range(HS):
            n0 = (L0 + k) * GP
            for n in range(n0 - WLAG * GP, n0 - (WLAG - 1) * GP):
                copy(n, 0).wait()
                copy(n, 1).wait()
            for n in range(n0, n0 + GP):
                copy(n, 0).start(priority=FG)
                copy(n + LAG, 1).start(priority=BG)
            if K0 <= k < K0 + len(work):
                work[k - K0]()
        return carry

    lax.fori_loop(0, HKV - 1, body, 0)
    state.update(issued=GA + L1, waited=GA + L1 - WLAG)

    g = HKV - 1
    ensure(GC - 1)
    scores(g, range(0, B // 2))
    advance(1)
    scores(g, range(B // 2, B))
    softmax()
    advance(2)
    values(g, range(B))
    advance(1)
    project(g)

    mod = mod_s[...]
    ga, sb, cb, gb = (mod[:, i * D:(i + 1) * D] for i in range(4))
    x2 = x_v[...].astype(F32) + ga * acc_s[...]
    h2 = _layernorm(x2) * (1.0 + cb) + sb
    h2b = h2.astype(BF16)
    wr = wr_v[...].astype(F32).reshape(1, D)
    rsel = jax.nn.sigmoid(jnp.sum(h2 * wr, axis=-1, keepdims=True))
    acc_s[...] = x2 + gb * h2
    h_s[...] = gb * rsel
    advance(1)
    ensure(last_of['G'])
    gate = _dot(h2b, wg_v[...])
    act_s[...] = gate * jax.nn.sigmoid(gate)
    advance(2)
    ensure(last_of['U'])
    actb_s[...] = (act_s[...] * _dot(h2b, wu_v[...])).astype(BF16)
    advance(1)
    outs = [pltpu.make_async_copy(out_v.at[:, pl.ds(c0, n)], out_hbm.at[:, pl.ds(c0, n)],
                                  sems.at[S_SMALL + i])
            for i, (c0, n) in enumerate(((0, DL), (DL, D - DL)))]
    for nm in order:
        r0, r1, f0, f1 = pieces[nm]
        advance(1)
        if nm in last_of:
            ensure(last_of[nm])
        else:
            assert state['waited'] == NG
            blk = wd_v.at[pl.ds(r0, r1 - r0), pl.ds(f0, f1 - f0)]
            pltpu.make_async_copy(blk, blk, sems.at[S_LAST + int(nm[1])]).wait()
        y = _dot_nt(actb_s[:, f0:f1], wd_v[r0:r1, f0:f1])
        val = acc_s[:, r0:r1] + h_s[:, r0:r1] * y
        if f1 < FF:
            acc_s[:, r0:r1] = val
        else:
            out_v[:, r0:r1] = val.astype(out_v.dtype)
        if nm == order[DL // 128 - 1]:
            outs[0].start()
    outs[1].start()
    for cp in outs:
        cp.wait()


@jax.jit
def pallas_adaLN_cond__sliding_block_cached__moe_arch_mod__decode_kernel(
    A_x: jax.Array,
    A_k_cache: jax.Array,
    A_v_cache: jax.Array,
    A_wq: jax.Array,
    A_wo: jax.Array,
    B_x: jax.Array,
    B_w_r: jax.Array,
    B_w_gate: jax.Array,
    B_w_up: jax.Array,
    B_w_down: jax.Array,
    c: jax.Array,
    w_mod: jax.Array,
):
    B, SQ, D = A_x.shape
    _, HKV, SK, _ = A_k_cache.shape
    FF = B_w_gate.shape[1]
    W = min(4096, max(256, SK // 4))
    assert SQ == 1 and HQ == 2 * HKV and B == 8 and W // 256 == B

    vm = pltpu.VMEM
    scratch = [
        vm((B, D), BF16), vm((B, D), BF16), vm((D,), BF16),
        vm((D, 6 * D), BF16), vm((D, HQ * DH), BF16), vm((D, HQ * DH), BF16),
        vm((D, FF), BF16), vm((D, FF), BF16), vm((D, FF), BF16),
        vm((2, B, W, DH), BF16), vm((2, B, W, DH), BF16),
        vm((B, 4 * D), F32),
        vm((B, D), F32),
        vm((HKV, 2 * B, DH), F32),
        vm((2 * B, W), F32),
        vm((2 * B, W), BF16),
        vm((2 * B, DH), F32),
        vm((2 * B, DH), F32),
        vm((B, D), F32),
        vm((B, FF), F32),
        vm((B, FF), BF16),
        vm((B, D), A_x.dtype),
        pltpu.SemaphoreType.DMA((S_RING + RS,)),
    ]
    out = pl.pallas_call(
        _kernel,
        out_shape=jax.ShapeDtypeStruct((B, D), A_x.dtype),
        in_specs=[pl.BlockSpec(memory_space=pl.ANY)] * 11,
        out_specs=pl.BlockSpec(memory_space=pl.ANY),
        scratch_shapes=scratch,
        compiler_params=pltpu.CompilerParams(
            vmem_limit_bytes=64 * 1024 * 1024,
            disable_bounds_checks=True,
            disable_semaphore_checks=True,
        ),
    )(A_x.reshape(B, D), A_k_cache, A_v_cache, A_wq, A_wo.T, B_w_r,
      B_w_gate, B_w_up, B_w_down.T, c, w_mod)
    return out.reshape(B, SQ, D)
```
